```python
import jax
import jax.numpy as jnp

def _softmax(x, axis=-1):
    return jax.nn.softmax(x, axis=axis)

def _gelu(x):
    return jax.nn.gelu(x, approximate=True)

def _silu(x):
    return jax.nn.silu(x)

def _sigmoid(x):
    return jax.nn.sigmoid(x)

def _layernorm(x, axis=-1, eps=1e-05):
    m = jnp.mean(x, axis=axis, keepdims=True)
    v = jnp.var(x, axis=axis, keepdims=True)
    return (x - m) / jnp.sqrt(v + eps)

def _scatter_add(tgt, idx, src, axis=0):
    return tgt.at[idx].add(src)

def _segment_sum(src, seg, n):
    return jax.ops.segment_sum(src, seg, n)

class _Rng:

    def __init__(self, key):
        self._k = key

    def _next(self):
        self._k, sub = jax.random.split(self._k)
        return sub

    def normal(self, shape):
        return jax.random.normal(self._next(), shape, dtype=jnp.bfloat16)

    def randint(self, lo, hi, shape):
        return jax.random.randint(self._next(), shape, lo, hi, dtype=jnp.int32)

    def uniform(self, shape, lo=0.0, hi=1.0):
        return jax.random.uniform(self._next(), shape, jnp.bfloat16, lo, hi)

    def permutation(self, n):
        return jax.random.permutation(self._next(), n)
kernel_name = 'adaLN_cond__compressed_kv_cla__mixer_s_mlp__decode'

def setup_inputs():
    _rng = _Rng(jax.random.key(int.from_bytes(__import__("os").urandom(4), "little")))
    _w = lambda a: (lambda t: t.astype(jnp.bfloat16) if jnp.issubdtype(t.dtype, jnp.floating) else t)(jnp.asarray(a))

    def _A_setup():
        B, H, Sq, Sk, D, M = (8, 32, 1, 4096, 128, 512)
        Dc = 4 * D
        return {'x': _w((lambda *s: _rng.normal(s) * 0.05)(B, Sq, M)), 'c_kv': _w((lambda *s: _rng.normal(s) * 0.05)(B, Sk, Dc)), 'w_q': _w((lambda *s: _rng.normal(s) * 0.05)(M, H, D) * M ** (-0.5)), 'w_uk': _w((lambda *s: _rng.normal(s) * 0.05)(Dc, H, D) * Dc ** (-0.5)), 'w_uv': _w((lambda *s: _rng.normal(s) * 0.05)(Dc, H, D) * Dc ** (-0.5)), 'w_o': _w((lambda *s: _rng.normal(s) * 0.05)(H, D, M) * (H * D) ** (-0.5))}
    _A_in = _A_setup()

    def _B_setup():
        B, S, D, F = (8, 1, 512, 1792)
        return {'x': _w((lambda *s: _rng.normal(s) * 0.05)(B, S, D)), 'w1': _w((lambda *s: _rng.normal(s) * 0.05)(D, D) * D ** (-0.5)), 'w2': _w((lambda *s: _rng.normal(s) * 0.05)(D, D) * D ** (-0.5)), 'w3': _w((lambda *s: _rng.normal(s) * 0.05)(D, F) * D ** (-0.5)), 'w4': _w((lambda *s: _rng.normal(s) * 0.05)(F, D) * F ** (-0.5))}
    _B_in = _B_setup()
    return {'A_x': _A_in['x'], 'A_c_kv': _A_in['c_kv'], 'A_w_q': _A_in['w_q'], 'A_w_uk': _A_in['w_uk'], 'A_w_uv': _A_in['w_uv'], 'A_w_o': _A_in['w_o'], 'B_x': _B_in['x'], 'B_w1': _B_in['w1'], 'B_w2': _B_in['w2'], 'B_w3': _B_in['w3'], 'B_w4': _B_in['w4'], 'c': _w((lambda *s: _rng.normal(s) * 0.05)(8, 512)), 'w_mod': _w((lambda *s: _rng.normal(s) * 0.05)(512, 6 * 512) * 512 ** (-0.5))}

def reference(A_x, A_c_kv, A_w_q, A_w_uk, A_w_uv, A_w_o, B_x, B_w1, B_w2, B_w3, B_w4, c, w_mod):

    def _A_ref(x, c_kv, w_q, w_uk, w_uv, w_o):
        B, Sq, M = (x.shape[0], x.shape[1], x.shape[2])
        Sk = c_kv.shape[1]
        H, D = (w_q.shape[1], w_q.shape[2])
        q = jnp.einsum('bqm,mhd->bhqd', x, w_q)
        k = jnp.einsum('bkc,chd->bhkd', c_kv, w_uk)
        v = jnp.einsum('bkc,chd->bhkd', c_kv, w_uv)
        scores = jnp.einsum('bhqd,bhkd->bhqk', q, k) * D ** (-0.5)
        off = Sk - Sq
        qi = jnp.arange(Sq)[:, None]
        kj = jnp.arange(Sk)[None, :]
        cmask = kj <= qi + off
        scores = jnp.where(cmask[None, None], scores, -1000000000.0)
        p = _softmax(scores, axis=-1)
        ctx = jnp.einsum('bhqk,bhkd->bhqd', p, v)
        return jnp.einsum('bhqd,hdm->bqm', ctx, w_o)

    def _B_ref(x, w1, w2, w3, w4):
        B, S, D = x.shape
        h = _gelu(_layernorm(x, axis=-1) @ w1)
        c = D // 4
        g0 = jnp.pad(h[:, :, 0 * c:1 * c], ((0, 0), (1, 0), (0, 0)))[:, :S, :]
        g1 = jnp.pad(h[:, :, 1 * c:2 * c], ((0, 0), (0, 1), (0, 0)))[:, 1:, :]
        g2 = jnp.pad(h[:, :, 2 * c:3 * c], ((0, 0), (2, 0), (0, 0)))[:, :S, :]
        g3 = jnp.pad(h[:, :, 3 * c:], ((0, 0), (0, 2), (0, 0)))[:, 2:, :]
        hs = jnp.concatenate([g0, g1, g2, g3], axis=-1) @ w2
        x1 = x + hs
        h2 = _gelu(_layernorm(x1, axis=-1) @ w3) @ w4
        return x1 + h2
    x = A_x
    mod = (_silu(c) @ w_mod).reshape(c.shape[0], 6, 1, -1)
    sa, ca, ga, sb, cb, gb = (mod[:, 0].copy(), mod[:, 1].copy(), mod[:, 2].copy(), mod[:, 3].copy(), mod[:, 4].copy(), mod[:, 5].copy())
    h = _layernorm(x, axis=-1) * (1 + ca) + sa
    x = x + ga * _A_ref(h, A_c_kv, A_w_q, A_w_uk, A_w_uv, A_w_o)
    h = _layernorm(x, axis=-1) * (1 + cb) + sb
    x = x + gb * _B_ref(h, B_w1, B_w2, B_w3, B_w4)
    return x
```

```python
import functools
import jax
import jax.numpy as jnp
from jax import lax
import jax.experimental.pallas as pl
import jax.experimental.pallas.tpu as pltpu

B, H, D, M, SK, DC, F = 8, 32, 128, 512, 4096, 512, 1792
NT = (((1,), (1,)), ((), ()))
BF, F32 = jnp.bfloat16, jnp.float32
NSTEP = 32

KC = 512
CFG = dict(L=10, L0=5, QS=3, PB=4, compute=True)


def _ln(x):
    m = jnp.mean(x, axis=-1, keepdims=True)
    d = x - m
    v = jnp.mean(d * d, axis=-1, keepdims=True)
    return d * lax.rsqrt(v + 1e-5)


def _head_pair(w_u32, i, j):
    view = w_u32.at[:, pl.ds(pl.multiple_of(4 * i, 4), 2048 - 12)]
    w = jnp.concatenate([view[k, pl.ds(j, 128, stride=16), :] for k in range(4)], axis=0)
    lo = pltpu.bitcast(w << 16, F32).astype(BF)
    hi = pltpu.bitcast(w & jnp.uint32(0xFFFF0000), F32).astype(BF)
    return lo, hi


def make_kernel(cfg):
    L, L0, QS, PB, compute = cfg["L"], cfg["L0"], cfg["QS"], cfg["PB"], cfg["compute"]
    off = cfg.get("off", "")
    PC = cfg.get("PC", 2)

    def kern(x_hbm, ckv_hbm, wq_hbm, wuk_hbm, wuv_hbm, wo_hbm, w3_hbm, w4_hbm, c_hbm, wmod_hbm, o_ref,
             x_v, c_v, wmod_v, wq_v, wuk_v, wuv_v, wo_v, w3_v, w4_v, kv_v,
             qa_v, qb_v, s_v, mx_v, l_v, acc_v, cc_v, ctx_v, sem, kv_sem, w4_sem):
        S_X, S_C, S_Q, S_UK, S_UV, S_O, S_3, S_MOD = range(8)

        def start(src, dst, s, pr):
            pltpu.make_async_copy(src, dst, s).start(priority=pr)

        def d_head(src, dst, s):
            def go(r, half, pr):
                ix = (pl.ds(2 * half, 2), pl.ds(pl.multiple_of(r * 64, 64), 64))
                start(src.at[ix], dst.at[ix], sem.at[s], pr)
            return go
        d_wq, d_wuk, d_wuv = d_head(wq_hbm, wq_v, S_Q), d_head(wuk_hbm, wuk_v, S_UK), d_head(wuv_hbm, wuv_v, S_UV)

        def d_wo(r, half, pr):
            ix = (pl.ds(2 * half, 2), pl.ds(pl.multiple_of(r * 16, 16), 16))
            start(wo_hbm.at[ix], wo_v.at[ix], sem.at[S_O], pr)

        def d_wmod(r, third, pr):
            rows = pl.ds(pl.multiple_of(r * 16, 16), 16)
            start(wmod_hbm.at[rows, pl.ds(third * 1024, 1024)], wmod_v.at[third, rows], sem.at[S_MOD + min(third, 1)], pr)

        def d_w3(r, half, pr):
            ix = (pl.ds(pl.multiple_of(r * 16, 16), 16), pl.ds(half * 896, 896))
            start(w3_hbm.at[ix], w3_v.at[ix], sem.at[S_3], pr)

        def d_w4(r, pr):
            ix = (slice(None), pl.ds(pl.multiple_of(r * 16, 16), 16))
            start(w4_hbm.at[ix], w4_v.at[ix], w4_sem.at[r // 8], pr)

        def d_kv(t, u):
            bb, half = (u % 8) // 2, u % 2
            rnd = 2 * t + u // 8
            g, j = rnd // 64, rnd % 64
            it = (rnd // 8) * 4 + bb
            src = ckv_hbm.at[pl.ds(g * 16 + bb * 4 + half * 2, 2), pl.ds(pl.multiple_of(j * 16, 16), 16)]
            dst = kv_v.at[it, pl.ds((rnd % 8) * 4 + half * 2, 2)]
            start(src, dst, kv_sem.at[it], u % 2)

        def wait_all(buf, s):
            pltpu.make_async_copy(buf, buf, s).wait()

        def loop(lo, hi, body):
            lax.fori_loop(lo, hi, lambda i, c: (body(i), c)[1], 0)

        def kv_slots(lo, hi):
            loop(lo, hi, lambda t: [d_kv(t, u) for u in range(16)])

        cx = pltpu.make_async_copy(x_hbm, x_v, sem.at[S_X])
        cc = pltpu.make_async_copy(c_hbm, c_v, sem.at[S_C])

        def p1(r):
            for k in range(2):
                d_wq(2 * r + k, 0, 0)
                d_wq(2 * r + k, 1, 1)
                d_wuk(2 * r + k, 0, 0)
                d_wuk(2 * r + k, 1, 1)
        def p1m(r):
            p1(2 * r)
            d_wmod(2 * r, 0, 0)
            d_wmod(2 * r + 1, 0, 1)
            p1(2 * r + 1)
        p1m(0)
        cc.start()
        cx.start(priority=1)
        loop(1, 16, p1m)
        kv_slots(0, L0)

        cc.wait()
        cx.wait()
        wait_all(wmod_v.at[0], sem.at[S_MOD])
        wait_all(wq_v, sem.at[S_Q])
        wait_all(wuk_v, sem.at[S_UK])
        wq_u = wq_v.bitcast(jnp.uint32)
        wuk_u = wuk_v.bitcast(jnp.uint32)
        wuv_u = wuv_v.bitcast(jnp.uint32)
        if compute:
            cf = c_v[...].astype(F32)
            sc = (cf * jax.nn.sigmoid(cf)).astype(BF)
            mod_a = jnp.dot(sc, wmod_v[0], preferred_element_type=F32) if 'm' not in off else wmod_v[0, 0:16, :].astype(F32)[0:8]
            x0 = x_v[...].astype(F32)
            h = (_ln(x0) * (1.0 + mod_a[:, M:]) + mod_a[:, :M]).astype(BF)

        def qstage(i):
            kv_slots(L0 + QS * i, L0 + QS * (i + 1))
            for j in range(4 if compute and 'q' not in off else 0):
                lo, hi = _head_pair(wq_u, i, j)
                q2 = jnp.dot(h, jnp.concatenate([lo, hi], axis=1), preferred_element_type=F32).astype(BF)
                for par, u in enumerate(_head_pair(wuk_u, i, j)):
                    qa = lax.dot_general(q2[:, par * D:(par + 1) * D], u, NT, preferred_element_type=F32)
                    qa = qa * (D ** -0.5)
                    row = pl.multiple_of((8 * i + 2 * j + par) * B, B)
                    for cb in range(4):
                        qa_v[cb, pl.ds(row, B), :] = qa[:, cb * 128:(cb + 1) * 128]
        loop(0, 4, qstage)
        if compute:
            for b in range(B):
                qb_v[b] = jnp.concatenate([qa_v[cb, pl.ds(b, H, stride=B), :] for cb in range(4)], axis=1).astype(BF)
            mx_v[...] = jnp.full(mx_v.shape, -jnp.inf, F32)
            l_v[...] = jnp.zeros(l_v.shape, F32)
            acc_v[...] = jnp.zeros(acc_v.shape, F32)

        def attn(it, qk, pv, issue):
            issue()
            if qk:
                wait_all(kv_v.at[it], kv_sem.at[it])
            if qk and compute and 'k' not in off:
                b = (it // NSTEP) * 4 + it % 4
                s = lax.dot_general(qb_v[b], kv_v[it].reshape(KC, DC), NT, preferred_element_type=F32)
                s_v[it] = s
                m = jnp.maximum(jnp.maximum(s[:, 0:128], s[:, 128:256]), jnp.maximum(s[:, 256:384], s[:, 384:512]))
                mx_v[b] = jnp.maximum(mx_v[b], m)
            if pv and compute and 'p' not in off:
                ip = it - NSTEP
                b = (ip // NSTEP) * 4 + ip % 4
                m = mx_v[b]
                p = jnp.exp(s_v[ip] - jnp.concatenate([m] * 4, axis=1))
                l_v[b] += (p[:, 0:128] + p[:, 128:256]) + (p[:, 256:384] + p[:, 384:512])
                acc_v[b] += jnp.dot(p.astype(BF), kv_v[ip].reshape(KC, DC), preferred_element_type=F32)

        def finish_max(g):
            for b in range(4 * g, 4 * g + 4):
                mx_v[b] = jnp.broadcast_to(jnp.max(mx_v[b], axis=-1, keepdims=True), (H, 128))

        def p3a(i):
            for k in range(4):
                d_wuv(4 * i + k, 0, 0)
                d_wuv(4 * i + k, 1, 1)
                if k % 2 == 0:
                    d_wo(2 * i + k // 2, 0, 0)
                    d_wo(2 * i + k // 2, 1, 1)
                else:
                    d_wmod(2 * i + k // 2, 1, 0)
                    d_wmod(2 * i + k // 2, 2, 1)

        def p3b(i):
            @pl.when(i < 4)
            def _():
                for k in range(8):
                    d_wo(32 + 8 * i + k, 0, 0)
                    d_wo(32 + 8 * i + k, 1, 1)

            @pl.when(i >= 4)
            def _():
                for k in range(8):
                    d_w3(8 * (i - 4) + k, 0, 0)
                    d_w3(8 * (i - 4) + k, 1, 1)

        def p3c(i):
            for k in range(7):
                d_w4(14 * i + 2 * k, 0)
                d_w4(14 * i + 2 * k + 1, 1)

        LA = L0 + 4 * QS
        NC = 2 * (LA - L)
        assert 0 <= NC <= NSTEP and L <= 16
        loop(0, NC // 2, lambda i: (attn(2 * i, True, False, lambda: [d_kv(LA + i, u) for u in range(16)]),
                                    attn(2 * i + 1, True, False, lambda: None)))
        loop(NC, NSTEP, lambda t: attn(t, True, False, lambda: [d_kv(t + L, u) for u in range(16)]))
        if compute:
            finish_max(0)
        loop(NSTEP, 2 * NSTEP - L, lambda t: attn(t, True, True, lambda: [d_kv(t + L, u) for u in range(16)]))
        loop(2 * NSTEP - L, 2 * NSTEP, lambda t: attn(t, True, True, lambda: p3a(t - (2 * NSTEP - L))))
        if compute:
            finish_max(1)
        n3 = 16 - L
        per = NSTEP // 4
        def pvl(i):
            loop(L + (n3 * i) // 4, L + (n3 * (i + 1)) // 4, p3a)
            loop(2 * NSTEP + per * i, 2 * NSTEP + per * (i + 1), lambda t: attn(t, False, True, lambda: None))
        loop(0, 4, pvl)

        loop(0, PB, p3b)
        if compute:
            for b in range(B):
                inv = 1.0 / jnp.sum(l_v[b], axis=-1, keepdims=True)
                cn = acc_v[b] * inv
                for cb in range(4):
                    cc_v[cb, pl.ds(b, H, stride=B), :] = cn[:, cb * 128:(cb + 1) * 128]
        wait_all(wmod_v.at[pl.ds(1, 2)], sem.at[S_MOD + 1])
        if compute:
            mod_b = jnp.dot(sc, wmod_v[1], preferred_element_type=F32) if 'm' not in off else wmod_v[1, 0:16, :].astype(F32)[0:8]
            mod_c = jnp.dot(sc, wmod_v[2], preferred_element_type=F32) if 'm' not in off else wmod_v[2, 0:16, :].astype(F32)[0:8]
        wait_all(wuv_v, sem.at[S_UV])

        def vstage(i):
            loop(PB + ((8 - PB) * i) // 4, PB + ((8 - PB) * (i + 1)) // 4, p3b)
            for j in range(4 if compute and 'v' not in off else 0):
                for par, u in enumerate(_head_pair(wuv_u, i, j)):
                    hh = 8 * i + 2 * j + par
                    row = pl.multiple_of(hh * B, B)
                    a = jnp.concatenate([cc_v[cb, pl.ds(row, B), :] for cb in range(4)], axis=1).astype(BF)
                    ctx_v[hh] = jnp.dot(a, u, preferred_element_type=F32)
        loop(0, 4, vstage)

        loop(0, PC, p3c)
        wait_all(wo_v, sem.at[S_O])
        if compute:
            ctx = jnp.concatenate([ctx_v[hh] for hh in range(H)], axis=1).astype(BF)
            att = jnp.dot(ctx, wo_v[...].reshape(H * D, M), preferred_element_type=F32) if 'o' not in off else ctx[:, :M].astype(F32)
            x1 = x0 + mod_b[:, :M] * att
            h2 = _ln(x1) * (1.0 + mod_c[:, :M]) + mod_b[:, M:]
            hn = _ln(h2).astype(BF)
        loop(PC, 4, p3c)
        wait_all(w3_v, sem.at[S_3])
        if compute:
            g = jnp.dot(hn, w3_v[...], preferred_element_type=F32) if '3' not in off else w3_v[0:16, :].astype(F32)[0:8]
            g = jax.nn.gelu(g, approximate=True).astype(BF)
            y = h2
        for k in range(7):
            wait_all(w4_v.at[:, pl.ds(k * 128, 128)], w4_sem.at[k])
            for half in range(2 if compute and '4' not in off else 0):
                c0 = half * 896 + k * 128
                y = y + jnp.dot(g[:, c0:c0 + 128], w4_v[half, pl.ds(k * 128, 128), :], preferred_element_type=F32)
        if compute:
            o_ref[...] = (x1 + mod_c[:, M:] * y).astype(o_ref.dtype)
        else:
            o_ref[...] = x_v[...]

    return kern


def build(cfg):
    @jax.jit
    def f(A_x, A_c_kv, A_w_q, A_w_uk, A_w_uv, A_w_o, B_x, B_w1, B_w2, B_w3, B_w4, c, w_mod):
        hbm = pl.BlockSpec(memory_space=pltpu.HBM)
        V = pltpu.VMEM
        return pl.pallas_call(
            make_kernel(cfg),
            out_shape=jax.ShapeDtypeStruct((B, M), A_x.dtype),
            in_specs=[hbm] * 10,
            out_specs=pl.BlockSpec(memory_space=pltpu.VMEM),
            scratch_shapes=[
                V((B, M), BF), V((B, M), BF), V((3, M, 2 * M), BF),
                V((4, 4096, D), BF), V((4, 4096, D), BF), V((4, 4096, D), BF), V((4, 1024, M), BF),
                V((M, F), BF), V((2, F // 2, M), BF), V((2 * NSTEP, 32, 16, DC), BF),
                V((4, H * B, 128), F32), V((B, H, DC), BF),
                V((2 * NSTEP, H, KC), F32), V((B, H, 128), F32), V((B, H, 128), F32), V((B, H, DC), F32),
                V((4, H * B, 128), F32), V((H, B, D), F32),
                pltpu.SemaphoreType.DMA((9,)), pltpu.SemaphoreType.DMA((2 * NSTEP,)), pltpu.SemaphoreType.DMA((7,)),
            ],
            compiler_params=pltpu.CompilerParams(vmem_limit_bytes=100 * 1024 * 1024, disable_bounds_checks=True),
        )(A_x.reshape(B, M), A_c_kv.reshape(32, 1024, DC), A_w_q.reshape(4, 4096, D), A_w_uk.reshape(4, 4096, D),
          A_w_uv.reshape(4, 4096, D), A_w_o.reshape(4, 1024, M), B_w3, B_w4.reshape(2, F // 2, M), c, w_mod).reshape(B, 1, M)
    return f


pallas_adaLN_cond__compressed_kv_cla__mixer_s_mlp__decode_kernel = build(CFG)
```

```python
import jax
import jax.numpy as jnp
from jax import lax
import jax.experimental.pallas as pl
import jax.experimental.pallas.tpu as pltpu

B, H, D, M, SK, DC, F = 8, 32, 128, 512, 4096, 512, 1792
KC = 512
NIT = B * SK // KC
NT = (((1,), (1,)), ((), ()))
BF, F32 = jnp.bfloat16, jnp.float32

CFG = dict(L0=4, QS=3, T=(16, 4, 44, 54), W=(3, 6), compute=True)


def _ln(x):
    d = x - jnp.mean(x, axis=-1, keepdims=True)
    return d * lax.rsqrt(jnp.mean(d * d, axis=-1, keepdims=True) + 1e-5)


def _head_pair(w_u32, i, j):
    view = w_u32.at[:, pl.ds(pl.multiple_of(4 * i, 4), 2048 - 12)]
    w = jnp.concatenate([view[k, pl.ds(j, 128, stride=16), :] for k in range(4)], axis=0)
    lo = pltpu.bitcast(w << 16, F32).astype(BF)
    hi = pltpu.bitcast(w & jnp.uint32(0xFFFF0000), F32).astype(BF)
    return lo, hi


def make_kernel(cfg):
    L0, QS, compute = cfg["L0"], cfg["QS"], cfg["compute"]
    T0, TV, T1, T2 = cfg["T"]
    W1, W2 = cfg['W']
    assert T0 + 4 * TV <= min(32, T1) and T1 <= T2 and 32 <= T2 <= 48 + 2 * W1
    dma, off = cfg.get("dma", True), cfg.get("off", "")
    L = L0 + 4 * QS
    assert L == 16 and L0 <= 8

    def kern(x_hbm, ckv_hbm, wq_hbm, wuk_hbm, wuv_hbm, wo_hbm, w3_hbm, w4_hbm, c_hbm, wmod_hbm, o_ref,
             kv_v, wq_v, wuk_v, wuv_v, wo_v, w3_v, w4_v, wmod_v, x_v, c_v,
             qa_v, qb_v, m_v, l_v, acc_v, cc_v, ctx_v, sem):
        def start(src, dst, s, pr):
            if dma:
                pltpu.make_async_copy(src, dst, sem.at[s]).start(priority=pr)

        def wait(buf, s):
            if dma:
                pltpu.make_async_copy(buf, buf, sem.at[s]).wait()

        def rows(r, n):
            return pl.ds(pl.multiple_of(r * n, n), n)

        def loop(lo, hi, body):
            if hi > lo:
                lax.fori_loop(lo, hi, lambda i, c: (body(i), c)[1], 0)

        def d_pair(src, dst, n, r, s):
            for half in range(2):
                ix = (pl.ds(2 * half, 2), rows(r, n))
                start(src.at[ix], dst.at[ix], s, half)

        def d_wmod(r, third, s, pr):
            start(wmod_hbm.at[rows(r, 16), pl.ds(third * 1024, 1024)], wmod_v.at[third, rows(r, 16)], s, pr)

        def kv_slot(t):
            for u in range(16):
                ix = (pl.ds(2 * (u % 8), 2), rows(2 * t + u // 8, 16))
                start(ckv_hbm.at[ix], kv_v.at[ix], (t // 8) % 2, u % 2)

        def uv_mod_slot(i):
            for k in range(4):
                d_pair(wuv_hbm, wuv_v, 64, 4 * i + k, i // 8)
                if k % 2 == 1:
                    d_wmod(2 * i + k // 2, 1, i // 8, 0)
                    d_wmod(2 * i + k // 2, 2, i // 8, 1)

        def o_quad(q):
            for e in range(2):
                d_pair(wo_hbm, wo_v, 16, 2 * q + e, 2)

        def w3_quad(q):
            for k in range(4):
                start(w3_hbm.at[k, rows(q, 8)], w3_v.at[k, rows(q, 8)], 0, k % 2)

        def w4_quad(s):
            def go(q):
                for k in range(4):
                    ix = (slice(None), rows(4 * q + k, 16))
                    start(w4_hbm.at[ix], w4_v.at[ix], s, k % 2)
            return go

        def tail_quads(lo, hi):
            for base, first, n, fn in ((0, 0, 32, o_quad), (32, 0, 16, w3_quad), (48, 0, 2 * W1, w4_quad(1)),
                                       (48 + 2 * W1, 2 * W1, 2 * (W2 - W1), w4_quad(2)),
                                       (48 + 2 * W2, 2 * W2, 2 * (7 - W2), w4_quad(3))):
                loop(max(lo, base) - base + first, min(hi, base + n) - base + first, fn)

        def p1(r):
            for k in range(4):
                d_pair(wq_hbm, wq_v, 64, 4 * r + k, 1)
                d_pair(wuk_hbm, wuk_v, 64, 4 * r + k, 1)
                if k == 1:
                    d_wmod(2 * r, 0, 1, 0)
                    d_wmod(2 * r + 1, 0, 1, 1)
        loop(0, 16, p1)
        start(c_hbm, c_v, 1, 0)
        start(x_hbm, x_v, 1, 1)
        loop(0, L0, kv_slot)

        for buf in (c_v, x_v, wmod_v.at[0], wq_v, wuk_v):
            wait(buf, 1)
        wq_u, wuk_u, wuv_u = (w.bitcast(jnp.uint32) for w in (wq_v, wuk_v, wuv_v))
        if compute:
            cf = c_v[...].astype(F32)
            sc = (cf * jax.nn.sigmoid(cf)).astype(BF)
            mod_a = jnp.dot(sc, wmod_v[0], preferred_element_type=F32)
            x0 = x_v[...].astype(F32)
            h = (_ln(x0) * (1.0 + mod_a[:, M:]) + mod_a[:, :M]).astype(BF)

        def qstage(i):
            lax.fori_loop(L0 + QS * i, L0 + QS * (i + 1), lambda t, c: (kv_slot(t), c)[1], 0)
            for j in range(4 if compute and 'q' not in off else 0):
                q2 = jnp.dot(h, jnp.concatenate(_head_pair(wq_u, i, j), axis=1),
                             preferred_element_type=F32).astype(BF)
                for par, u in enumerate(_head_pair(wuk_u, i, j)):
                    qa = lax.dot_general(q2[:, par * D:(par + 1) * D], u, NT, preferred_element_type=F32)
                    qa = qa * (D ** -0.5)
                    for cb in range(4):
                        qa_v[cb, rows(8 * i + 2 * j + par, B), :] = qa[:, cb * 128:(cb + 1) * 128]
        loop(0, 4, qstage)
        if compute:
            for b in range(B):
                qb_v[b] = jnp.concatenate([qa_v[cb, pl.ds(b, H, stride=B), :] for cb in range(4)],
                                          axis=1).astype(BF)
            m_v[...] = jnp.full(m_v.shape, -jnp.inf, F32)
            l_v[...] = jnp.zeros(l_v.shape, F32)
            acc_v[...] = jnp.zeros(acc_v.shape, F32)

        def attn(it, issue):
            sweep, b = it // B, it % B

            @pl.when(b == 0)
            def _():
                wait(kv_v.at[:, rows(sweep, KC // 2)], sweep % 2)

            issue()
            if compute and 'k' not in off:
                kv = kv_v.at[rows(b, 2), rows(sweep, KC // 2)]
                s = lax.dot_general(qb_v[b], kv[...].reshape(KC, DC), NT, preferred_element_type=F32)
                m_old = m_v[b]
                m_new = jnp.maximum(m_old, jnp.max(s, axis=-1, keepdims=True))
                alpha = jnp.exp(m_old - m_new)
                p = jnp.exp(s - jnp.concatenate([m_new] * 4, axis=1))
                m_v[b] = m_new
                l_v[b] = alpha * l_v[b] + ((p[:, 0:128] + p[:, 128:256]) + (p[:, 256:384] + p[:, 384:512]))
                pv = jnp.dot(p.astype(BF), kv[...].reshape(KC, DC), preferred_element_type=F32)
                acc_v[b] = jnp.concatenate([alpha] * 4, axis=1) * acc_v[b] + pv
        loop(0, NIT - L, lambda it: attn(it, lambda: kv_slot(it + L)))
        loop(NIT - L, NIT, lambda it: attn(it, lambda: uv_mod_slot(it - (NIT - L))))

        if compute:
            for b in range(B):
                cn = acc_v[b] / jnp.sum(l_v[b], axis=-1, keepdims=True)
                for cb in range(4):
                    cc_v[cb, pl.ds(b, H, stride=B), :] = cn[:, cb * 128:(cb + 1) * 128]
        tail_quads(0, T0)
        for s in range(2):
            wait(wuv_v.at[:, rows(s, 2048)], s)
            wait(wmod_v.at[pl.ds(1, 2), rows(s, M // 2)], s)

        def vstage(i):
            lax.fori_loop(T0 + TV * i, T0 + TV * (i + 1), lambda q, c: (o_quad(q), c)[1], 0)
            for j in range(4 if compute and 'v' not in off else 0):
                for par, u in enumerate(_head_pair(wuv_u, i, j)):
                    hh = 8 * i + 2 * j + par
                    a = jnp.concatenate([cc_v[cb, rows(hh, B), :] for cb in range(4)], axis=1).astype(BF)
                    ctx_v[hh] = jnp.dot(a, u, preferred_element_type=F32)
        loop(0, 4, vstage)

        tail_quads(T0 + 4 * TV, T1)
        if compute:
            mod_b = jnp.dot(sc, wmod_v[1], preferred_element_type=F32)
            mod_c = jnp.dot(sc, wmod_v[2], preferred_element_type=F32)
        tail_quads(T1, T2)
        wait(wo_v, 2)
        if compute:
            ctx = jnp.concatenate([ctx_v[hh] for hh in range(H)], axis=1).astype(BF)
            att = jnp.dot(ctx, wo_v[...].reshape(H * D, M), preferred_element_type=F32)
            x1 = x0 + mod_b[:, :M] * att
            h2 = _ln(x1) * (1.0 + mod_c[:, :M]) + mod_b[:, M:]
            hn = _ln(h2).astype(BF)
        tail_quads(T2, 62)
        wait(w3_v, 0)
        if compute:
            g = jnp.dot(hn, w3_v[...].reshape(M, F), preferred_element_type=F32)
            g = jax.nn.gelu(g, approximate=True).astype(BF)
            y = h2
        for s, lo, hi in ((1, 0, W1), (2, W1, W2), (3, W2, 7)):
            wait(w4_v.at[:, pl.ds(lo * 128, (hi - lo) * 128)], s)
            for half in range(2 if compute else 0):
                c0 = half * (F // 2)
                y = y + jnp.dot(g[:, c0 + lo * 128:c0 + hi * 128], w4_v[half, lo * 128:hi * 128, :],
                                preferred_element_type=F32)
        if compute:
            o_ref[...] = (x1 + mod_c[:, M:] * y).astype(o_ref.dtype)
        else:
            o_ref[...] = x_v[...]

    return kern


def build(cfg):
    @jax.jit
    def f(A_x, A_c_kv, A_w_q, A_w_uk, A_w_uv, A_w_o, B_x, B_w1, B_w2, B_w3, B_w4, c, w_mod):
        V = pltpu.VMEM
        out = pl.pallas_call(
            make_kernel(cfg),
            out_shape=jax.ShapeDtypeStruct((B, M), A_x.dtype),
            in_specs=[pl.BlockSpec(memory_space=pltpu.HBM)] * 10,
            out_specs=pl.BlockSpec(memory_space=pltpu.VMEM),
            scratch_shapes=[
                V((2 * B, SK // 2, DC), BF),
                V((4, 4096, D), BF), V((4, 4096, D), BF), V((4, 4096, D), BF), V((4, 1024, M), BF),
                V((4, M // 4, F), BF), V((2, F // 2, M), BF), V((3, M, 2 * M), BF), V((B, M), BF), V((B, M), BF),
                V((4, H * B, 128), F32), V((B, H, DC), BF),
                V((B, H, 128), F32), V((B, H, 128), F32), V((B, H, DC), F32),
                V((4, H * B, 128), F32), V((H, B, D), F32),
                pltpu.SemaphoreType.DMA((4,)),
            ],
            compiler_params=pltpu.CompilerParams(vmem_limit_bytes=100 * 1024 * 1024,
                                                 disable_bounds_checks=True),
        )(A_x.reshape(B, M), A_c_kv.reshape(2 * B, SK // 2, DC), A_w_q.reshape(4, 4096, D),
          A_w_uk.reshape(4, 4096, D), A_w_uv.reshape(4, 4096, D), A_w_o.reshape(4, 1024, M),
          B_w3.reshape(4, M // 4, F), B_w4.reshape(2, F // 2, M), c, w_mod)
        return out.reshape(B, 1, M)
    return f


pallas_adaLN_cond__compressed_kv_cla__mixer_s_mlp__decode_kernel = build(CFG)
```

```python
import jax
import jax.numpy as jnp
from jax import lax
import jax.experimental.pallas as pl
import jax.experimental.pallas.tpu as pltpu

B, H, D, M, SK, DC, F = 8, 32, 128, 512, 4096, 512, 1792
KC = 512
NIT = B * SK // KC
NT = (((1,), (1,)), ((), ()))
BF, F32 = jnp.bfloat16, jnp.float32

CFG = dict(L0=4, QS=3, T=(20, 3, 40, 54), W=(10, 13), compute=True)


def _ln(x):
    d = x - jnp.mean(x, axis=-1, keepdims=True)
    return d * lax.rsqrt(jnp.mean(d * d, axis=-1, keepdims=True) + 1e-5)


def _head_pair(w_u32, i, j):
    view = w_u32.at[:, pl.ds(pl.multiple_of(4 * i, 4), 2048 - 12)]
    w = jnp.concatenate([view[k, pl.ds(j, 128, stride=16), :] for k in range(4)], axis=0)
    lo = pltpu.bitcast(w << 16, F32).astype(BF)
    hi = pltpu.bitcast(w & jnp.uint32(0xFFFF0000), F32).astype(BF)
    return lo, hi


def make_kernel(cfg):
    L0, QS, compute = cfg["L0"], cfg["QS"], cfg["compute"]
    T0, TV, T1, T2 = cfg["T"]
    W1, W2 = cfg["W"]
    W4_PARTS = ((1, 0, W1), (2, W1, W2), (3, W2, 14))
    assert T0 + 4 * TV <= min(32, T1) and T1 <= T2 and 32 <= T2 <= 48 + 2 * (W1 - 7)
    LP = cfg.get('LP', L0)
    dma, off = cfg.get("dma", True), cfg.get("off", "")
    L = L0 + 4 * QS
    assert 8 <= L <= 16 and L0 <= 8

    def kern(x_hbm, ckv_hbm, wq_hbm, wuk_hbm, wuv_hbm, wo_hbm, w3_hbm, w4_hbm, c_hbm, wmod_hbm, o_ref,
             kv_v, wq_v, wuk_v, wuv_v, wo_v, w3_v, w4_v, wmod_v, x_v, c_v,
             qa_v, qb_v, m_v, l_v, acc_v, cc_v, ctx_v, sem):
        def start(src, dst, s, pr):
            if dma:
                pltpu.make_async_copy(src, dst, sem.at[s]).start(priority=pr)

        def wait(buf, s):
            if dma:
                pltpu.make_async_copy(buf, buf, sem.at[s]).wait()

        def rows(r, n):
            return pl.ds(pl.multiple_of(r * n, n), n)

        def loop(lo, hi, body):
            if hi > lo:
                lax.fori_loop(lo, hi, lambda i, c: (body(i), c)[1], 0)

        def d_pair(src, dst, n, r, s):
            for half in range(2):
                ix = (pl.ds(2 * half, 2), rows(r, n))
                start(src.at[ix], dst.at[ix], s, half)

        def d_wmod(r, third, s, pr):
            start(wmod_hbm.at[rows(r, 16), pl.ds(third * 1024, 1024)], wmod_v.at[third, rows(r, 16)], s, pr)

        def kv_slot(t):
            for u in range(16):
                ix = (pl.ds(2 * (u % 8), 2), rows(2 * t + u // 8, 16))
                start(ckv_hbm.at[ix], kv_v.at[ix], (t // 8) % 2, u % 2)

        def uv_mod_slot(i):
            for k in range(4):
                d_pair(wuv_hbm, wuv_v, 64, 4 * i + k, i // 8)
                if k % 2 == 1:
                    d_wmod(2 * i + k // 2, 1, i // 8, 0)
                    d_wmod(2 * i + k // 2, 2, i // 8, 1)

        def o_quad(q):
            for e in range(2):
                d_pair(wo_hbm, wo_v, 16, 2 * q + e, 2)

        def w3_quad(q):
            for k in range(4):
                ix = ((q % 2) * 4 + k, rows(q // 2, 8))
                start(w3_hbm.at[ix], w3_v.at[ix], 0, k % 2)

        def w4_quad(q):
            for k in range(4):
                e = 2 * q + k // 2
                blk, r = (e % 7, e // 7) if k % 2 == 0 else (7 + e // 4, e % 4)
                s = [p for p, lo, hi in W4_PARTS if lo <= blk < hi][0]
                ix = (blk, pl.ds(32 * r, 32))
                start(w4_hbm.at[ix], w4_v.at[ix], s, k % 2)

        def tail_quads(lo, hi):
            for base, n, fn in ((0, 32, o_quad), (32, 16, w3_quad)):
                loop(max(lo, base) - base, min(hi, base + n) - base, fn)
            for q in range(max(lo, 48), hi):
                w4_quad(q - 48)

        def p1(r):
            for k in range(4):
                d_pair(wq_hbm, wq_v, 64, 4 * r + k, 1)
                d_pair(wuk_hbm, wuk_v, 64, 4 * r + k, 1)
                if k == 1:
                    d_wmod(2 * r, 0, 1, 0)
                    d_wmod(2 * r + 1, 0, 1, 1)
        loop(0, 16, p1)
        start(c_hbm, c_v, 1, 0)
        start(x_hbm, x_v, 1, 1)
        loop(0, LP, kv_slot)

        for buf in (c_v, x_v, wmod_v.at[0], wq_v, wuk_v):
            wait(buf, 1)
        wq_u, wuk_u, wuv_u = (w.bitcast(jnp.uint32) for w in (wq_v, wuk_v, wuv_v))
        if compute:
            cf = c_v[...].astype(F32)
            sc = (cf * jax.nn.sigmoid(cf)).astype(BF)
            mod_a = jnp.dot(sc, wmod_v[0], preferred_element_type=F32)
            x0 = x_v[...].astype(F32)
            h = (_ln(x0) * (1.0 + mod_a[:, M:]) + mod_a[:, :M]).astype(BF)

        def qstage(i):
            lax.fori_loop(jnp.maximum(LP, L0 + QS * i), L0 + QS * (i + 1), lambda t, c: (kv_slot(t), c)[1], 0)
            for j in range(4 if compute and 'q' not in off else 0):
                q2 = jnp.dot(h, jnp.concatenate(_head_pair(wq_u, i, j), axis=1),
                             preferred_element_type=F32).astype(BF)
                for par, u in enumerate(_head_pair(wuk_u, i, j)):
                    qa = lax.dot_general(q2[:, par * D:(par + 1) * D], u, NT, preferred_element_type=F32)
                    qa = qa * (D ** -0.5)
                    for cb in range(4):
                        qa_v[cb, rows(8 * i + 2 * j + par, B), :] = qa[:, cb * 128:(cb + 1) * 128]
        loop(0, 4, qstage)
        if compute:
            for b in range(B):
                qb_v[b] = jnp.concatenate([qa_v[cb, pl.ds(b, H, stride=B), :] for cb in range(4)],
                                          axis=1).astype(BF)
            m_v[...] = jnp.full(m_v.shape, -jnp.inf, F32)
            l_v[...] = jnp.zeros(l_v.shape, F32)
            acc_v[...] = jnp.zeros(acc_v.shape, F32)

        def attn(it, issue):
            sweep, b = it // B, it % B

            @pl.when(b == 0)
            def _():
                wait(kv_v.at[:, rows(sweep, KC // 2)], sweep % 2)

            issue()
            if compute and 'k' not in off:
                kv = kv_v.at[rows(b, 2), rows(sweep, KC // 2)]
                s = lax.dot_general(qb_v[b], kv[...].reshape(KC, DC), NT, preferred_element_type=F32)
                m_old = m_v[b]
                m_new = jnp.maximum(m_old, jnp.max(s, axis=-1, keepdims=True))
                alpha = jnp.exp(m_old - m_new)
                p = jnp.exp(s - jnp.concatenate([m_new] * 4, axis=1))
                m_v[b] = m_new
                l_v[b] = alpha * l_v[b] + ((p[:, 0:128] + p[:, 128:256]) + (p[:, 256:384] + p[:, 384:512]))
                pv = jnp.dot(p.astype(BF), kv[...].reshape(KC, DC), preferred_element_type=F32)
                acc_v[b] = jnp.concatenate([alpha] * 4, axis=1) * acc_v[b] + pv
        loop(0, NIT - L, lambda it: attn(it, lambda: kv_slot(it + L)))
        loop(NIT - L, NIT, lambda it: attn(it, lambda: uv_mod_slot(it - (NIT - L))))

        loop(L, 16, uv_mod_slot)
        if compute:
            for b in range(B):
                cn = acc_v[b] / jnp.sum(l_v[b], axis=-1, keepdims=True)
                for cb in range(4):
                    cc_v[cb, pl.ds(b, H, stride=B), :] = cn[:, cb * 128:(cb + 1) * 128]
        tail_quads(0, T0)
        for s in range(2):
            wait(wuv_v.at[:, rows(s, 2048)], s)
            wait(wmod_v.at[pl.ds(1, 2), rows(s, M // 2)], s)

        def vstage(i):
            lax.fori_loop(T0 + TV * i, T0 + TV * (i + 1), lambda q, c: (o_quad(q), c)[1], 0)
            for j in range(4 if compute and 'v' not in off else 0):
                for par, u in enumerate(_head_pair(wuv_u, i, j)):
                    hh = 8 * i + 2 * j + par
                    a = jnp.concatenate([cc_v[cb, rows(hh, B), :] for cb in range(4)], axis=1).astype(BF)
                    ctx_v[hh] = jnp.dot(a, u, preferred_element_type=F32)
        loop(0, 4, vstage)

        tail_quads(T0 + 4 * TV, T1)
        if compute:
            mod_b = jnp.dot(sc, wmod_v[1], preferred_element_type=F32)
            mod_c = jnp.dot(sc, wmod_v[2], preferred_element_type=F32)
        tail_quads(T1, T2)
        wait(wo_v, 2)
        if compute:
            ctx = jnp.concatenate([ctx_v[hh] for hh in range(H)], axis=1).astype(BF)
            att = jnp.dot(ctx, wo_v[...].reshape(H * D, M), preferred_element_type=F32)
            x1 = x0 + mod_b[:, :M] * att
            h2 = _ln(x1) * (1.0 + mod_c[:, :M]) + mod_b[:, M:]
            hn = _ln(h2).astype(BF)
        tail_quads(T2, 62)
        wait(w3_v, 0)
        if compute:
            g = jnp.dot(hn, w3_v[...].reshape(M, F), preferred_element_type=F32)
            g = jax.nn.gelu(g, approximate=True).astype(BF)
            y = h2
        for s, lo, hi in W4_PARTS:
            wait(w4_v.at[pl.ds(lo, hi - lo)], s)
            if compute:
                y = y + jnp.dot(g[:, lo * 128:hi * 128], w4_v[lo:hi].reshape((hi - lo) * 128, M),
                                preferred_element_type=F32)
        if compute:
            o_ref[...] = (x1 + mod_c[:, M:] * y).astype(o_ref.dtype)
        else:
            o_ref[...] = x_v[...]

    return kern


def build(cfg):
    @jax.jit
    def f(A_x, A_c_kv, A_w_q, A_w_uk, A_w_uv, A_w_o, B_x, B_w1, B_w2, B_w3, B_w4, c, w_mod):
        V = pltpu.VMEM
        out = pl.pallas_call(
            make_kernel(cfg),
            out_shape=jax.ShapeDtypeStruct((B, M), A_x.dtype),
            in_specs=[pl.BlockSpec(memory_space=pltpu.HBM)] * 10,
            out_specs=pl.BlockSpec(memory_space=pltpu.VMEM),
            scratch_shapes=[
                V((2 * B, SK // 2, DC), BF),
                V((4, 4096, D), BF), V((4, 4096, D), BF), V((4, 4096, D), BF), V((4, 1024, M), BF),
                V((8, M // 8, F), BF), V((F // 128, 128, M), BF), V((3, M, 2 * M), BF), V((B, M), BF), V((B, M), BF),
                V((4, H * B, 128), F32), V((B, H, DC), BF),
                V((B, H, 128), F32), V((B, H, 128), F32), V((B, H, DC), F32),
                V((4, H * B, 128), F32), V((H, B, D), F32),
                pltpu.SemaphoreType.DMA((4,)),
            ],
            compiler_params=pltpu.CompilerParams(vmem_limit_bytes=100 * 1024 * 1024,
                                                 disable_bounds_checks=True),
        )(A_x.reshape(B, M), A_c_kv.reshape(2 * B, SK // 2, DC), A_w_q.reshape(4, 4096, D),
          A_w_uk.reshape(4, 4096, D), A_w_uv.reshape(4, 4096, D), A_w_o.reshape(4, 1024, M),
          B_w3.reshape(8, M // 8, F), B_w4.reshape(F // 128, 128, M), c, w_mod)
        return out.reshape(B, 1, M)
    return f


pallas_adaLN_cond__compressed_kv_cla__mixer_s_mlp__decode_kernel = build(CFG)
```

```python
import jax
import jax.numpy as jnp
from jax import lax
import jax.experimental.pallas as pl
import jax.experimental.pallas.tpu as pltpu

B, H, D, M, SK, DC, F = 8, 32, 128, 512, 4096, 512, 1792
KC = 512
NIT = B * SK // KC
NT = (((1,), (1,)), ((), ()))
BF, F32 = jnp.bfloat16, jnp.float32

CFG = dict(L0=4, QS=3, T=(6, 10, 2, 12), LP=6, W=(10, 13), compute=True)


def _ln(x):
    d = x - jnp.mean(x, axis=-1, keepdims=True)
    return d * lax.rsqrt(jnp.mean(d * d, axis=-1, keepdims=True) + 1e-5)


def _head_pair(w_u32, i, j):
    view = w_u32.at[:, pl.ds(pl.multiple_of(4 * i, 4), 2048 - 12)]
    w = jnp.concatenate([view[k, pl.ds(j, 128, stride=16), :] for k in range(4)], axis=0)
    lo = pltpu.bitcast(w << 16, F32).astype(BF)
    hi = pltpu.bitcast(w & jnp.uint32(0xFFFF0000), F32).astype(BF)
    return lo, hi


def make_kernel(cfg):
    L0, QS, compute = cfg["L0"], cfg["QS"], cfg["compute"]
    T0, TV, T1, T2 = cfg["T"]
    W1, W2 = cfg["W"]
    W4_PARTS = ((2, 0, W1), (3, W1, W2), (0, W2, 14))
    assert T0 + TV <= 16 and T1 <= 2 * (W1 - 7) and T1 <= T2 <= 2 * (W2 - 7)
    LP = cfg.get('LP', L0)
    dma, off = cfg.get("dma", True), cfg.get("off", "")
    L = L0 + 4 * QS
    assert 8 <= L <= 16 and L0 <= 8

    def kern(x_hbm, ckv_hbm, wq_hbm, wuk_hbm, wuv_hbm, wo_hbm, w3_hbm, w4_hbm, c_hbm, wmod_hbm, o_ref,
             kv_v, wq_v, wuk_v, wuv_v, wo_v, w3_v, w4_v, wma_v, wmb_v, x_v, c_v,
             qa_v, qb_v, m_v, l_v, acc_v, cc_v, ctx_v, sem):
        def start(src, dst, s, pr):
            if dma:
                pltpu.make_async_copy(src, dst, sem.at[s]).start(priority=pr)

        def wait(buf, s):
            if dma:
                pltpu.make_async_copy(buf, buf, sem.at[s]).wait()

        def rows(r, n):
            return pl.ds(pl.multiple_of(r * n, n), n)

        def loop(lo, hi, body):
            if hi > lo:
                lax.fori_loop(lo, hi, lambda i, c: (body(i), c)[1], 0)

        def d_pair(src, dst, n, r, s, low=0):
            for half in range(2):
                ix = (pl.ds(2 * half, 2), rows(r, n))
                start(src.at[ix], dst.at[ix], s, max(half, low))

        def kv_slot(t):
            for u in range(16):
                ix = (pl.ds(2 * (u % 8), 2), rows(2 * t + u // 8, 16))
                start(ckv_hbm.at[ix], kv_v.at[ix], (t // 8) % 2, u % 2)

        def uv_o_slot(i):
            for k in range(8):
                r, half = 4 * i + k // 2, pl.ds(2 * (k % 2), 2)
                start(wuv_hbm.at[half, rows(r, 64)], wuv_v.at[half, rows(r, 64)], 2, 0)
                start(wo_hbm.at[half, rows(r, 16)], wo_v.at[half, rows(r, 16)], 3, 1)

        def mod_w3_quad(q):
            for k in range(4):
                ix = ((q % 2) * 4 + k, rows(q // 2, 8))
                start(wmod_hbm.at[ix + (pl.ds(2 * M, 4 * M),)], wmb_v.at[ix], 0, 0)
                start(w3_hbm.at[ix], w3_v.at[ix], 1, 1)

        def w4_quad(q):
            for k in range(4):
                e = 2 * q + k // 2
                blk, r = (e % 7, e // 7) if k % 2 == 0 else (7 + e // 4, e % 4)
                s = [p for p, lo, hi in W4_PARTS if lo <= blk < hi][0]
                ix = (blk, pl.ds(32 * r, 32))
                start(w4_hbm.at[ix], w4_v.at[ix], s, k % 2)

        def p1(r, low=0):
            for k in range(4):
                d_pair(wq_hbm, wq_v, 64, 4 * r + k, 1, low)
                d_pair(wuk_hbm, wuk_v, 64, 4 * r + k, 1, low)
                if k == 1:
                    for e in range(2):
                        ix = ((r % 4) * 2 + e, rows(r // 4, 16))
                        start(wmod_hbm.at[ix + (pl.ds(0, 2 * M),)], wma_v.at[ix], 1, e)
        PF = cfg.get('pf', 0)
        loop(0, PF, lambda r: p1(r, 1))
        loop(PF, 16, p1)
        start(c_hbm, c_v, 1, 0)
        start(x_hbm, x_v, 1, 1)
        loop(0, LP, kv_slot)

        for buf in (c_v, x_v, wma_v, wq_v, wuk_v):
            wait(buf, 1)
        wq_u, wuk_u, wuv_u = (w.bitcast(jnp.uint32) for w in (wq_v, wuk_v, wuv_v))
        if compute:
            cf = c_v[...].astype(F32)
            sc = (cf * jax.nn.sigmoid(cf)).astype(BF)
            mod_a = jnp.dot(sc, wma_v[...].reshape(M, 2 * M), preferred_element_type=F32)
            x0 = x_v[...].astype(F32)
            h = (_ln(x0) * (1.0 + mod_a[:, M:]) + mod_a[:, :M]).astype(BF)

        def qstage(i):
            lax.fori_loop(jnp.maximum(LP, L0 + QS * i), L0 + QS * (i + 1), lambda t, c: (kv_slot(t), c)[1], 0)
            for j in range(4 if compute and 'q' not in off else 0):
                q2 = jnp.dot(h, jnp.concatenate(_head_pair(wq_u, i, j), axis=1),
                             preferred_element_type=F32).astype(BF)
                for par, u in enumerate(_head_pair(wuk_u, i, j)):
                    qa = lax.dot_general(q2[:, par * D:(par + 1) * D], u, NT, preferred_element_type=F32)
                    qa = qa * (D ** -0.5)
                    for cb in range(4):
                        qa_v[cb, rows(8 * i + 2 * j + par, B), :] = qa[:, cb * 128:(cb + 1) * 128]
        loop(0, 4, qstage)
        if compute:
            for b in range(B):
                qb_v[b] = jnp.concatenate([qa_v[cb, pl.ds(b, H, stride=B), :] for cb in range(4)],
                                          axis=1).astype(BF)
            m_v[...] = jnp.full(m_v.shape, -jnp.inf, F32)
            l_v[...] = jnp.zeros(l_v.shape, F32)
            acc_v[...] = jnp.zeros(acc_v.shape, F32)

        def attn(it, issue):
            sweep, b = it // B, it % B

            @pl.when(b == 0)
            def _():
                wait(kv_v.at[:, rows(sweep, KC // 2)], sweep % 2)

            issue()
            if compute and 'k' not in off:
                kv = kv_v.at[rows(b, 2), rows(sweep, KC // 2)]
                s = lax.dot_general(qb_v[b], kv[...].reshape(KC, DC), NT, preferred_element_type=F32)
                m_old = m_v[b]
                m_new = jnp.maximum(m_old, jnp.max(s, axis=-1, keepdims=True))
                alpha = jnp.exp(m_old - m_new)
                p = jnp.exp(s - jnp.concatenate([m_new] * 4, axis=1))
                m_v[b] = m_new
                l_v[b] = alpha * l_v[b] + ((p[:, 0:128] + p[:, 128:256]) + (p[:, 256:384] + p[:, 384:512]))
                pv = jnp.dot(p.astype(BF), kv[...].reshape(KC, DC), preferred_element_type=F32)
                acc_v[b] = jnp.concatenate([alpha] * 4, axis=1) * acc_v[b] + pv
        loop(0, NIT - L, lambda it: attn(it, lambda: kv_slot(it + L)))
        loop(NIT - L, NIT, lambda it: attn(it, lambda: uv_o_slot(it - (NIT - L))))

        loop(L, 16, uv_o_slot)
        if compute:
            for b in range(B):
                cn = acc_v[b] / jnp.sum(l_v[b], axis=-1, keepdims=True)
                for cb in range(4):
                    cc_v[cb, pl.ds(b, H, stride=B), :] = cn[:, cb * 128:(cb + 1) * 128]
        loop(0, T0, mod_w3_quad)
        wait(wuv_v, 2)

        def vstage(i):
            lax.fori_loop(T0 + (TV * i) // 4, T0 + (TV * (i + 1)) // 4, lambda q, c: (mod_w3_quad(q), c)[1], 0)
            for j in range(4 if compute and 'v' not in off else 0):
                for par, u in enumerate(_head_pair(wuv_u, i, j)):
                    hh = 8 * i + 2 * j + par
                    a = jnp.concatenate([cc_v[cb, rows(hh, B), :] for cb in range(4)], axis=1).astype(BF)
                    ctx_v[hh] = jnp.dot(a, u, preferred_element_type=F32)
        loop(0, 4, vstage)

        loop(T0 + TV, 16, mod_w3_quad)
        for q in range(0, T1):
            w4_quad(q)
        wait(wo_v, 3)
        if compute:
            ctx = jnp.concatenate([ctx_v[hh] for hh in range(H)], axis=1).astype(BF)
            att = jnp.dot(ctx, wo_v[...].reshape(H * D, M), preferred_element_type=F32)
        for q in range(T1, T2):
            w4_quad(q)
        wait(wmb_v, 0)
        for q in range(T2, 14):
            w4_quad(q)
        if compute:
            mod_bc = jnp.dot(sc, wmb_v[...].reshape(M, 4 * M), preferred_element_type=F32)
            mod_b, mod_c = mod_bc[:, :2 * M], mod_bc[:, 2 * M:]
            x1 = x0 + mod_b[:, :M] * att
            h2 = _ln(x1) * (1.0 + mod_c[:, :M]) + mod_b[:, M:]
            hn = _ln(h2).astype(BF)
        wait(w3_v, 1)
        if compute:
            g = jnp.dot(hn, w3_v[...].reshape(M, F), preferred_element_type=F32)
            g = jax.nn.gelu(g, approximate=True).astype(BF)
            y = h2
        for s, lo, hi in W4_PARTS:
            wait(w4_v.at[pl.ds(lo, hi - lo)], s)
            if compute:
                y = y + jnp.dot(g[:, lo * 128:hi * 128], w4_v[lo:hi].reshape((hi - lo) * 128, M),
                                preferred_element_type=F32)
        if compute:
            res = (x1 + mod_c[:, M:] * y).astype(o_ref.dtype)
        else:
            res = x_v[...]
        if cfg.get("mo"):
            c_v[...] = res
            cp = pltpu.make_async_copy(c_v, o_ref, sem.at[0])
            cp.start()
            cp.wait()
        else:
            o_ref[...] = res

    return kern


def build(cfg):
    @jax.jit
    def f(A_x, A_c_kv, A_w_q, A_w_uk, A_w_uv, A_w_o, B_x, B_w1, B_w2, B_w3, B_w4, c, w_mod):
        V = pltpu.VMEM
        out = pl.pallas_call(
            make_kernel(cfg),
            out_shape=jax.ShapeDtypeStruct((B, M), A_x.dtype),
            in_specs=[pl.BlockSpec(memory_space=pltpu.HBM)] * 10,
            out_specs=pl.BlockSpec(memory_space=pltpu.HBM if cfg.get('mo') else pltpu.VMEM),
            scratch_shapes=[
                V((2 * B, SK // 2, DC), BF),
                V((4, 4096, D), BF), V((4, 4096, D), BF), V((4, 4096, D), BF), V((4, 1024, M), BF),
                V((8, M // 8, F), BF), V((F // 128, 128, M), BF), V((8, M // 8, 2 * M), BF), V((8, M // 8, 4 * M), BF), V((B, M), BF), V((B, M), BF),
                V((4, H * B, 128), F32), V((B, H, DC), BF),
                V((B, H, 128), F32), V((B, H, 128), F32), V((B, H, DC), F32),
                V((4, H * B, 128), F32), V((H, B, D), F32),
                pltpu.SemaphoreType.DMA((4,)),
            ],
            compiler_params=pltpu.CompilerParams(vmem_limit_bytes=100 * 1024 * 1024,
                                                 disable_bounds_checks=True),
        )(A_x.reshape(B, M), A_c_kv.reshape(2 * B, SK // 2, DC), A_w_q.reshape(4, 4096, D),
          A_w_uk.reshape(4, 4096, D), A_w_uv.reshape(4, 4096, D), A_w_o.reshape(4, 1024, M),
          B_w3.reshape(8, M // 8, F), B_w4.reshape(F // 128, 128, M), c, w_mod.reshape(8, M // 8, 6 * M))
        return out.reshape(B, 1, M)
    return f


pallas_adaLN_cond__compressed_kv_cla__mixer_s_mlp__decode_kernel = build(CFG)
```

```python
import jax
import jax.numpy as jnp
from jax import lax
import jax.experimental.pallas as pl
import jax.experimental.pallas.tpu as pltpu

B, H, D, M, SK, DC, F = 8, 32, 128, 512, 4096, 512, 1792
KC = 512
NIT = B * SK // KC
NT = (((1,), (1,)), ((), ()))
BF, F32 = jnp.bfloat16, jnp.float32

CFG = dict(L0=4, QS=3, T=(6, 10, 2, 12), LP=6, TS=516, QP=(7, 10, 13), QU=4, W=(10, 13), compute=True)


def _ln(x):
    d = x - jnp.mean(x, axis=-1, keepdims=True)
    return d * lax.rsqrt(jnp.mean(d * d, axis=-1, keepdims=True) + 1e-5)


def _gather_heads(w_ref, t_ref, i, stride):
    words = pltpu.bitcast(w_ref[i // 4, pl.ds(pl.multiple_of((i % 4) * 1024, 1024), 1024), :], jnp.uint32)
    dst = t_ref.at[pl.ds(pl.multiple_of(32 * i, 32), 15 * stride + 32)]
    for r in range(32):
        dst[pl.ds(r, 16, stride=stride), :] = words[16 * r:16 * r + 16]


def _head_pair(t_ref, s, stride):
    w = t_ref[pl.ds(pl.multiple_of(s * stride, stride & -stride & 31 or 32), 512), :]
    lo = pltpu.bitcast(w << 16, F32).astype(BF)
    hi = pltpu.bitcast(w & jnp.uint32(0xFFFF0000), F32).astype(BF)
    return lo, hi


def make_kernel(cfg):
    L0, QS, compute = cfg["L0"], cfg["QS"], cfg["compute"]
    T0, TV, T1, T2 = cfg["T"]
    W1, W2 = cfg["W"]
    W4_PARTS = ((2, 0, W1), (3, W1, W2), (0, W2, 14))
    assert T0 + TV <= 16 and T1 <= 2 * (W1 - 7) and T1 <= T2 <= 2 * (W2 - 7)
    LP = cfg.get('LP', L0)
    dma, off = cfg.get("dma", True), cfg.get("off", "")
    TS, QP, QU = cfg['TS'], cfg['QP'], cfg['QU']
    L = cfg.get('L', 16)
    assert 8 <= L <= 16 and L0 <= 8

    def kern(x_hbm, ckv_hbm, wq_hbm, wuk_hbm, wuv_hbm, wo_hbm, w3_hbm, w4_hbm, c_hbm, wmod_hbm, o_ref,
             kv_v, wq_v, wuk_v, wuv_v, wo_v, w3_v, w4_v, wma_v, wmb_v, x_v, c_v,
             ta_v, tb_v, qa_v, qb_v, m_v, l_v, acc_v, cc_v, ctx_v, sem):
        def start(src, dst, s, pr):
            if dma:
                pltpu.make_async_copy(src, dst, sem.at[s]).start(priority=pr)

        def wait(buf, s):
            if dma:
                pltpu.make_async_copy(buf, buf, sem.at[s]).wait()

        def rows(r, n):
            return pl.ds(pl.multiple_of(r * n, n), n)

        def loop(lo, hi, body):
            if hi > lo:
                lax.fori_loop(lo, hi, lambda i, c: (body(i), c)[1], 0)

        def d_pair(src, dst, n, r, s, low=0):
            for half in range(2):
                ix = (pl.ds(2 * half, 2), rows(r, n))
                start(src.at[ix], dst.at[ix], s, max(half, low))

        def kv_slot(t):
            for u in range(16):
                ix = (pl.ds(2 * (u % 8), 2), rows(2 * t + u // 8, 16))
                start(ckv_hbm.at[ix], kv_v.at[ix], (t // 8) % 2, u % 2)

        def uv_o_slot(i):
            for k in range(8):
                r, half = 4 * i + k // 2, pl.ds(2 * (k % 2), 2)
                start(wuv_hbm.at[half, rows(r, 64)], wuv_v.at[half, rows(r, 64)], 2, 0)
                start(wo_hbm.at[half, rows(r, 16)], wo_v.at[half, rows(r, 16)], 3, 1)

        def mod_w3_quad(q):
            for k in range(4):
                ix = ((q % 2) * 4 + k, rows(q // 2, 8))
                start(wmod_hbm.at[ix + (pl.ds(2 * M, 4 * M),)], wmb_v.at[ix], 0, 0)
                start(w3_hbm.at[ix], w3_v.at[ix], 1, 1)

        def w4_quad(q):
            for k in range(4):
                e = 2 * q + k // 2
                blk, r = (e % 7, e // 7) if k % 2 == 0 else (7 + e // 4, e % 4)
                s = [p for p, lo, hi in W4_PARTS if lo <= blk < hi][0]
                ix = (blk, pl.ds(32 * r, 32))
                start(w4_hbm.at[ix], w4_v.at[ix], s, k % 2)

        def p1(r, low=0):
            for k in range(4):
                d_pair(wq_hbm, wq_v, 64, 4 * r + k, 1, low)
                d_pair(wuk_hbm, wuk_v, 64, 4 * r + k, 1, low)
                if k == 1:
                    for e in range(2):
                        ix = ((r % 4) * 2 + e, rows(r // 4, 16))
                        start(wmod_hbm.at[ix + (pl.ds(0, 2 * M),)], wma_v.at[ix], 1, e)
        PF = cfg.get('pf', 0)
        loop(0, PF, lambda r: p1(r, 1))
        loop(PF, 16, p1)
        start(c_hbm, c_v, 1, 0)
        start(x_hbm, x_v, 1, 1)
        loop(0, LP, kv_slot)

        for buf in (c_v, x_v, wma_v, wq_v, wuk_v):
            wait(buf, 1)
        if compute:
            cf = c_v[...].astype(F32)
            sc = (cf * jax.nn.sigmoid(cf)).astype(BF)
            mod_a = jnp.dot(sc, wma_v[...].reshape(M, 2 * M), preferred_element_type=F32)
            x0 = x_v[...].astype(F32)
            h = (_ln(x0) * (1.0 + mod_a[:, M:]) + mod_a[:, :M]).astype(BF)

        def relayout(w_ref, t_ref, lo, hi):
            if compute:
                loop(lo, hi, lambda i: _gather_heads(w_ref, t_ref, i, TS))

        def qstage(s):
            q2 = jnp.dot(h, jnp.concatenate(_head_pair(ta_v, s, TS), axis=1), preferred_element_type=F32).astype(BF)
            for par, u in enumerate(_head_pair(tb_v, s, TS)):
                qa = lax.dot_general(q2[:, par * D:(par + 1) * D], u, NT, preferred_element_type=F32)
                qa = qa * (D ** -0.5)
                for cb in range(4):
                    qa_v[cb, rows(2 * s + par, B), :] = qa[:, cb * 128:(cb + 1) * 128]

        loop(LP, QP[0], kv_slot)
        relayout(wq_v, ta_v, 0, 16)
        loop(QP[0], QP[1], kv_slot)
        relayout(wuk_v, tb_v, 0, 16)
        loop(QP[1], QP[2], kv_slot)
        if compute:
            loop(0, 16 // QU, lambda i: [lax.fori_loop(QP[2] + i // 2, QP[2] + (i + 1) // 2, lambda t, c: (kv_slot(t), c)[1], 0)]
                 + [qstage(QU * i + j) for j in range(QU)])
        else:
            loop(QP[2], QP[2] + 8 // QU, kv_slot)
        loop(QP[2] + 8 // QU, L, kv_slot)
        if compute:
            for b in range(B):
                qb_v[b] = jnp.concatenate([qa_v[cb, pl.ds(b, H, stride=B), :] for cb in range(4)],
                                          axis=1).astype(BF)
            m_v[...] = jnp.full(m_v.shape, -jnp.inf, F32)
            l_v[...] = jnp.zeros(l_v.shape, F32)
            acc_v[...] = jnp.zeros(acc_v.shape, F32)

        def attn(it, issue):
            sweep, b = it // B, it % B

            @pl.when(b == 0)
            def _():
                wait(kv_v.at[:, rows(sweep, KC // 2)], sweep % 2)

            issue()
            if compute and 'k' not in off:
                kv = kv_v.at[rows(b, 2), rows(sweep, KC // 2)]
                s = lax.dot_general(qb_v[b], kv[...].reshape(KC, DC), NT, preferred_element_type=F32)
                m_old = m_v[b]
                m_new = jnp.maximum(m_old, jnp.max(s, axis=-1, keepdims=True))
                alpha = jnp.exp(m_old - m_new)
                p = jnp.exp(s - jnp.concatenate([m_new] * 4, axis=1))
                m_v[b] = m_new
                l_v[b] = alpha * l_v[b] + ((p[:, 0:128] + p[:, 128:256]) + (p[:, 256:384] + p[:, 384:512]))
                pv = jnp.dot(p.astype(BF), kv[...].reshape(KC, DC), preferred_element_type=F32)
                acc_v[b] = jnp.concatenate([alpha] * 4, axis=1) * acc_v[b] + pv
        loop(0, NIT - L, lambda it: attn(it, lambda: kv_slot(it + L)))
        loop(NIT - L, NIT, lambda it: attn(it, lambda: uv_o_slot(it - (NIT - L))))

        loop(L, 16, uv_o_slot)
        if compute:
            for b in range(B):
                cn = acc_v[b] / jnp.sum(l_v[b], axis=-1, keepdims=True)
                for cb in range(4):
                    cc_v[cb, pl.ds(b, H, stride=B), :] = cn[:, cb * 128:(cb + 1) * 128]
        loop(0, T0, mod_w3_quad)
        wait(wuv_v, 2)

        def vstage(s):
            for par, u in enumerate(_head_pair(ta_v, s, TS)):
                a = jnp.concatenate([cc_v[cb, rows(2 * s + par, B), :] for cb in range(4)], axis=1).astype(BF)
                ctx_v[2 * s + par] = jnp.dot(a, u, preferred_element_type=F32)

        relayout(wuv_v, ta_v, 0, 16)
        loop(T0, T0 + TV, mod_w3_quad)
        if compute:
            loop(0, 16 // QU, lambda i: [vstage(QU * i + j) for j in range(QU)])
        loop(T0 + TV, 16, mod_w3_quad)
        for q in range(0, T1):
            w4_quad(q)
        wait(wo_v, 3)
        if compute:
            ctx = jnp.concatenate([ctx_v[hh] for hh in range(H)], axis=1).astype(BF)
            att = jnp.dot(ctx, wo_v[...].reshape(H * D, M), preferred_element_type=F32)
        for q in range(T1, T2):
            w4_quad(q)
        wait(wmb_v, 0)
        for q in range(T2, 14):
            w4_quad(q)
        if compute:
            mod_bc = jnp.dot(sc, wmb_v[...].reshape(M, 4 * M), preferred_element_type=F32)
            mod_b, mod_c = mod_bc[:, :2 * M], mod_bc[:, 2 * M:]
            x1 = x0 + mod_b[:, :M] * att
            h2 = _ln(x1) * (1.0 + mod_c[:, :M]) + mod_b[:, M:]
            hn = _ln(h2).astype(BF)
        wait(w3_v, 1)
        if compute:
            g = jnp.dot(hn, w3_v[...].reshape(M, F), preferred_element_type=F32)
            g = jax.nn.gelu(g, approximate=True).astype(BF)
            y = h2
        for s, lo, hi in W4_PARTS:
            wait(w4_v.at[pl.ds(lo, hi - lo)], s)
            if compute:
                y = y + jnp.dot(g[:, lo * 128:hi * 128], w4_v[lo:hi].reshape((hi - lo) * 128, M),
                                preferred_element_type=F32)
        if compute:
            res = (x1 + mod_c[:, M:] * y).astype(o_ref.dtype)
        else:
            res = x_v[...]
        if cfg.get("mo"):
            c_v[...] = res
            cp = pltpu.make_async_copy(c_v, o_ref, sem.at[0])
            cp.start()
            cp.wait()
        else:
            o_ref[...] = res

    return kern


def build(cfg):
    @jax.jit
    def f(A_x, A_c_kv, A_w_q, A_w_uk, A_w_uv, A_w_o, B_x, B_w1, B_w2, B_w3, B_w4, c, w_mod):
        V = pltpu.VMEM
        out = pl.pallas_call(
            make_kernel(cfg),
            out_shape=jax.ShapeDtypeStruct((B, M), A_x.dtype),
            in_specs=[pl.BlockSpec(memory_space=pltpu.HBM)] * 10,
            out_specs=pl.BlockSpec(memory_space=pltpu.HBM if cfg.get('mo') else pltpu.VMEM),
            scratch_shapes=[
                V((2 * B, SK // 2, DC), BF),
                V((4, 4096, D), BF), V((4, 4096, D), BF), V((4, 4096, D), BF), V((4, 1024, M), BF),
                V((8, M // 8, F), BF), V((F // 128, 128, M), BF), V((8, M // 8, 2 * M), BF), V((8, M // 8, 4 * M), BF), V((B, M), BF), V((B, M), BF),
                V((16 * cfg['TS'], D), jnp.uint32), V((16 * cfg['TS'], D), jnp.uint32),
                V((4, H * B, 128), F32), V((B, H, DC), BF),
                V((B, H, 128), F32), V((B, H, 128), F32), V((B, H, DC), F32),
                V((4, H * B, 128), F32), V((H, B, D), F32),
                pltpu.SemaphoreType.DMA((4,)),
            ],
            compiler_params=pltpu.CompilerParams(vmem_limit_bytes=100 * 1024 * 1024,
                                                 disable_bounds_checks=True),
        )(A_x.reshape(B, M), A_c_kv.reshape(2 * B, SK // 2, DC), A_w_q.reshape(4, 4096, D),
          A_w_uk.reshape(4, 4096, D), A_w_uv.reshape(4, 4096, D), A_w_o.reshape(4, 1024, M),
          B_w3.reshape(8, M // 8, F), B_w4.reshape(F // 128, 128, M), c, w_mod.reshape(8, M // 8, 6 * M))
        return out.reshape(B, 1, M)
    return f


pallas_adaLN_cond__compressed_kv_cla__mixer_s_mlp__decode_kernel = build(CFG)
```

```python
import jax
import jax.numpy as jnp
from jax import lax
import jax.experimental.pallas as pl
import jax.experimental.pallas.tpu as pltpu

B, H, D, M, SK, DC, F = 8, 32, 128, 512, 4096, 512, 1792
BF, F32 = jnp.bfloat16, jnp.float32
NT = (((1,), (1,)), ((), ()))

KC = 512
NBLK = B * SK // KC
LEAD = 16
TS = 516
W4_PARTS = ((2, 0, 10), (3, 10, 13), (0, 13, 14))


def _ln(x):
    d = x - jnp.mean(x, axis=-1, keepdims=True)
    return d * lax.rsqrt(jnp.mean(d * d, axis=-1, keepdims=True) + 1e-5)


def _dot(a, b):
    return jnp.dot(a, b, preferred_element_type=F32)


def _rows(i, n):
    return pl.ds(pl.multiple_of(i * n, n), n)


def _loop(lo, hi, body):
    lax.fori_loop(lo, hi, lambda i, carry: (body(i), carry)[1], 0)


def _gather_heads(w_ref, t_ref):
    def step(i):
        words = pltpu.bitcast(w_ref[i // 4, _rows(i % 4, 32 * H), :], jnp.uint32)
        dst = t_ref.at[pl.ds(pl.multiple_of(32 * i, 32), 16 * TS + 32)]
        for r in range(32):
            dst[pl.ds(r, 16, stride=TS), :] = words[16 * r:16 * r + 16]
    _loop(0, 16, step)


def _head_pair(t_ref, s):
    w = t_ref[pl.ds(pl.multiple_of(s * TS, 4), 512), :]
    even = pltpu.bitcast(w << 16, F32).astype(BF)
    odd = pltpu.bitcast(w & jnp.uint32(0xFFFF0000), F32).astype(BF)
    return even, odd


def _kernel(x_hbm, kv_hbm, wq_hbm, wuk_hbm, wuv_hbm, wo_hbm, w3_hbm, w4_hbm, c_hbm, wmod_hbm, o_ref,
            kv_v, wq_v, wuk_v, wuv_v, wo_v, w3_v, w4_v, wma_v, wmb_v, x_v, c_v,
            ta_v, tb_v, qa_v, qb_v, m_v, l_v, acc_v, cc_v, ctx_v, sem):
    def start(src, dst, s, queue):
        pltpu.make_async_copy(src, dst, sem.at[s]).start(priority=queue)

    def wait(buf, s):
        pltpu.make_async_copy(buf, buf, sem.at[s]).wait()

    def head_slot(i):
        for k in range(4):
            for src, dst in ((wq_hbm, wq_v), (wuk_hbm, wuk_v)):
                for half in range(2):
                    ix = (pl.ds(2 * half, 2), _rows(4 * i + k, 64))
                    start(src.at[ix], dst.at[ix], 1, half)
            if k == 1:
                for e in range(2):
                    ix = ((i % 4) * 2 + e, _rows(i // 4, 16))
                    start(wmod_hbm.at[ix + (pl.ds(0, 2 * M),)], wma_v.at[ix], 1, e)

    def kv_slot(t):
        for u in range(16):
            ix = (pl.ds(2 * (u % B), 2), _rows(2 * t + u // B, 16))
            start(kv_hbm.at[ix], kv_v.at[ix], (t // B) % 2, u % 2)

    def uv_o_slot(i):
        for k in range(8):
            r, half = 4 * i + k // 2, pl.ds(2 * (k % 2), 2)
            start(wuv_hbm.at[half, _rows(r, 64)], wuv_v.at[half, _rows(r, 64)], 2, 0)
            start(wo_hbm.at[half, _rows(r, 16)], wo_v.at[half, _rows(r, 16)], 3, 1)

    def mod_w3_step(i):
        for k in range(4):
            ix = ((i % 2) * 4 + k, _rows(i // 2, 8))
            start(wmod_hbm.at[ix + (pl.ds(2 * M, 4 * M),)], wmb_v.at[ix], 0, 0)
            start(w3_hbm.at[ix], w3_v.at[ix], 1, 1)

    def w4_steps(lo, hi):
        for e in range(lo, hi):
            for queue, (blk, r) in enumerate(((e % 7, e // 7), (7 + e // 4, e % 4))):
                s, = [s for s, first, last in W4_PARTS if first <= blk < last]
                ix = (blk, pl.ds(32 * r, 32))
                start(w4_hbm.at[ix], w4_v.at[ix], s, queue)

    _loop(0, 16, head_slot)
    start(c_hbm, c_v, 1, 0)
    start(x_hbm, x_v, 1, 1)
    _loop(0, 6, kv_slot)
    for buf in (c_v, x_v, wma_v, wq_v, wuk_v):
        wait(buf, 1)

    cond = c_v[...].astype(F32)
    cond = (cond * jax.nn.sigmoid(cond)).astype(BF)
    mod = _dot(cond, wma_v[...].reshape(M, 2 * M))
    shift_a, scale_a = mod[:, :M], mod[:, M:]
    x0 = x_v[...].astype(F32)
    h = (_ln(x0) * (1.0 + scale_a) + shift_a).astype(BF)

    _loop(6, 7, kv_slot)
    _gather_heads(wq_v, ta_v)
    _loop(7, 10, kv_slot)
    _gather_heads(wuk_v, tb_v)
    _loop(10, 13, kv_slot)

    def query(i):
        _loop(13 + i // 2, 13 + (i + 1) // 2, kv_slot)
        for j in range(4):
            s = 4 * i + j
            q = _dot(h, jnp.concatenate(_head_pair(ta_v, s), axis=1)).astype(BF)
            for e, wuk in enumerate(_head_pair(tb_v, s)):
                qa = lax.dot_general(q[:, e * D:(e + 1) * D], wuk, NT, preferred_element_type=F32)
                qa = qa * (D ** -0.5)
                for cb in range(4):
                    qa_v[cb, _rows(2 * s + e, B), :] = qa[:, cb * 128:(cb + 1) * 128]
    _loop(0, 4, query)
    _loop(15, LEAD, kv_slot)

    for b in range(B):
        qb_v[b] = jnp.concatenate([qa_v[cb, pl.ds(b, H, stride=B), :] for cb in range(4)], axis=1).astype(BF)
    m_v[...] = jnp.full(m_v.shape, -jnp.inf, F32)
    l_v[...] = jnp.zeros(l_v.shape, F32)
    acc_v[...] = jnp.zeros(acc_v.shape, F32)

    def attend(i, refill):
        sweep, b = i // B, i % B

        @pl.when(b == 0)
        def _():
            wait(kv_v.at[:, _rows(sweep, KC // 2)], sweep % 2)

        refill()
        kv = kv_v.at[_rows(b, 2), _rows(sweep, KC // 2)]
        s = lax.dot_general(qb_v[b], kv[...].reshape(KC, DC), NT, preferred_element_type=F32)
        m_old = m_v[b]
        m_new = jnp.maximum(m_old, jnp.max(s, axis=-1, keepdims=True))
        alpha = jnp.exp(m_old - m_new)
        p = jnp.exp(s - jnp.concatenate([m_new] * 4, axis=1))
        m_v[b] = m_new
        l_v[b] = alpha * l_v[b] + ((p[:, 0:128] + p[:, 128:256]) + (p[:, 256:384] + p[:, 384:512]))
        pv = _dot(p.astype(BF), kv[...].reshape(KC, DC))
        acc_v[b] = jnp.concatenate([alpha] * 4, axis=1) * acc_v[b] + pv
    _loop(0, NBLK - LEAD, lambda i: attend(i, lambda: kv_slot(i + LEAD)))
    _loop(NBLK - LEAD, NBLK, lambda i: attend(i, lambda: uv_o_slot(i - (NBLK - LEAD))))

    for b in range(B):
        latent = acc_v[b] / jnp.sum(l_v[b], axis=-1, keepdims=True)
        for cb in range(4):
            cc_v[cb, pl.ds(b, H, stride=B), :] = latent[:, cb * 128:(cb + 1) * 128]

    _loop(0, 6, mod_w3_step)
    wait(wuv_v, 2)
    _gather_heads(wuv_v, ta_v)
    _loop(6, 16, mod_w3_step)

    def value(i):
        for j in range(4):
            s = 4 * i + j
            for e, wuv in enumerate(_head_pair(ta_v, s)):
                latent = jnp.concatenate([cc_v[cb, _rows(2 * s + e, B), :] for cb in range(4)], axis=1)
                ctx_v[2 * s + e] = _dot(latent.astype(BF), wuv)
    _loop(0, 4, value)

    w4_steps(0, 4)
    wait(wo_v, 3)
    ctx = jnp.concatenate([ctx_v[i] for i in range(H)], axis=1).astype(BF)
    att = _dot(ctx, wo_v[...].reshape(H * D, M))

    w4_steps(4, 24)
    wait(wmb_v, 0)
    w4_steps(24, 28)
    mod = _dot(cond, wmb_v[...].reshape(M, 4 * M))
    gate_a, shift_b, scale_b, gate_b = (mod[:, i * M:(i + 1) * M] for i in range(4))
    x1 = x0 + gate_a * att

    y = _ln(x1) * (1.0 + scale_b) + shift_b
    yn = _ln(y).astype(BF)
    wait(w3_v, 1)
    g = jax.nn.gelu(_dot(yn, w3_v[...].reshape(M, F)), approximate=True).astype(BF)
    for s, first, last in W4_PARTS:
        wait(w4_v.at[pl.ds(first, last - first)], s)
        y = y + _dot(g[:, first * 128:last * 128], w4_v[first:last].reshape((last - first) * 128, M))
    o_ref[...] = (x1 + gate_b * y).astype(o_ref.dtype)


@jax.jit
def pallas_adaLN_cond__compressed_kv_cla__mixer_s_mlp__decode_kernel(
    A_x: jax.Array,
    A_c_kv: jax.Array,
    A_w_q: jax.Array,
    A_w_uk: jax.Array,
    A_w_uv: jax.Array,
    A_w_o: jax.Array,
    B_x: jax.Array,
    B_w1: jax.Array,
    B_w2: jax.Array,
    B_w3: jax.Array,
    B_w4: jax.Array,
    c: jax.Array,
    w_mod: jax.Array,
):
    assert A_x.shape == (B, 1, M) and A_c_kv.shape == (B, SK, DC) and B_w3.shape == (M, F)
    vmem = pltpu.VMEM
    out = pl.pallas_call(
        _kernel,
        out_shape=jax.ShapeDtypeStruct((B, M), A_x.dtype),
        in_specs=[pl.BlockSpec(memory_space=pltpu.HBM)] * 10,
        out_specs=pl.BlockSpec(memory_space=pltpu.VMEM),
        scratch_shapes=[
            vmem((2 * B, SK // 2, DC), BF),
            vmem((4, M * H // 4, D), BF), vmem((4, DC * H // 4, D), BF),
            vmem((4, DC * H // 4, D), BF), vmem((4, H * D // 4, M), BF),
            vmem((8, M // 8, F), BF), vmem((F // 128, 128, M), BF),
            vmem((8, M // 8, 2 * M), BF), vmem((8, M // 8, 4 * M), BF),
            vmem((B, M), BF), vmem((B, M), BF),
            vmem((16 * TS + 512, D), jnp.uint32), vmem((16 * TS + 512, D), jnp.uint32),
            vmem((4, (H + 1) * B, 128), F32), vmem((B, H, DC), BF),
            vmem((B, H, 128), F32), vmem((B, H, 128), F32), vmem((B, H, DC), F32),
            vmem((4, (H + 1) * B, 128), F32), vmem((H, B, D), F32),
            pltpu.SemaphoreType.DMA((4,)),
        ],
        compiler_params=pltpu.CompilerParams(vmem_limit_bytes=100 * 1024 * 1024),
    )(
        A_x.reshape(B, M),
        A_c_kv.reshape(2 * B, SK // 2, DC),
        A_w_q.reshape(4, M * H // 4, D),
        A_w_uk.reshape(4, DC * H // 4, D),
        A_w_uv.reshape(4, DC * H // 4, D),
        A_w_o.reshape(4, H * D // 4, M),
        B_w3.reshape(8, M // 8, F),
        B_w4.reshape(F // 128, 128, M),
        c,
        w_mod.reshape(8, M // 8, 6 * M),
    )
    return out.reshape(B, 1, M)
```

```python
import jax
import jax.numpy as jnp
import numpy as np
from jax import lax
import jax.experimental.pallas as pl
import jax.experimental.pallas.tpu as pltpu

B, H, D, M, SK, DC, F = 8, 32, 128, 512, 4096, 512, 1792
BF, F32 = jnp.bfloat16, jnp.float32
NT = (((1,), (1,)), ((), ()))

KC = 512
NBLK = B * SK // KC
LEAD = 16
TS = 516
W4_PARTS = ((2, 0, 10), (3, 10, 13), (0, 13, 14))


def _ln(x):
    d = x - jnp.mean(x, axis=-1, keepdims=True)
    return d * lax.rsqrt(jnp.mean(d * d, axis=-1, keepdims=True) + 1e-5)


def _dot(a, b):
    return jnp.dot(a, b, preferred_element_type=F32)


def _rows(i, n):
    return pl.ds(pl.multiple_of(i * n, n), n)


def _loop(lo, hi, body):
    lax.fori_loop(lo, hi, lambda i, carry: (body(i), carry)[1], 0)


def _gather_heads(w_ref, t_ref):
    def step(i):
        words = pltpu.bitcast(w_ref[i // 4, _rows(i % 4, 32 * H), :], jnp.uint32)
        dst = t_ref.at[pl.ds(pl.multiple_of(32 * i, 32), 16 * TS + 32)]
        for r in range(32):
            dst[pl.ds(r, 16, stride=TS), :] = words[16 * r:16 * r + 16]
    _loop(0, 16, step)


def _head_pair(t_ref, s):
    w = t_ref[pl.ds(pl.multiple_of(s * TS, 4), 512), :]
    even = pltpu.bitcast(w << 16, F32).astype(BF)
    odd = pltpu.bitcast(w & np.uint32(0xFFFF0000), F32).astype(BF)
    return even, odd


def _kernel(x_hbm, kv_hbm, wq_hbm, wuk_hbm, wuv_hbm, wo_hbm, w3_hbm, w4_hbm, c_hbm, wmod_hbm, o_ref,
            kv_v, wq_v, wuk_v, wuv_v, wo_v, w3_v, w4_v, wma_v, wmb_v, x_v, c_v,
            ta_v, tb_v, qa_v, qb_v, m_v, l_v, acc_v, cc_v, ctx_v, sem):
    def start(src, dst, s, queue):
        pltpu.make_async_copy(src, dst, sem.at[s]).start(priority=queue)

    def wait(buf, s):
        pltpu.make_async_copy(buf, buf, sem.at[s]).wait()

    def head_slot(i, low=0):
        for k in range(4):
            for src, dst in ((wq_hbm, wq_v), (wuk_hbm, wuk_v)):
                for half in range(2):
                    ix = (pl.ds(2 * half, 2), _rows(4 * i + k, 64))
                    start(src.at[ix], dst.at[ix], 1, max(half, low))
            if k == 1:
                for e in range(2):
                    ix = ((i % 4) * 2 + e, _rows(i // 4, 16))
                    start(wmod_hbm.at[ix + (pl.ds(0, 2 * M),)], wma_v.at[ix], 1, max(e, low))

    def kv_slot(t):
        for u in range(16):
            ix = (pl.ds(2 * (u % B), 2), _rows(2 * t + u // B, 16))
            start(kv_hbm.at[ix], kv_v.at[ix], (t // B) % 2, u % 2)

    def uv_o_slot(i):
        for k in range(8):
            r, half = 4 * i + k // 2, pl.ds(2 * (k % 2), 2)
            start(wuv_hbm.at[half, _rows(r, 64)], wuv_v.at[half, _rows(r, 64)], 2, 0)
            start(wo_hbm.at[half, _rows(r, 16)], wo_v.at[half, _rows(r, 16)], 3, 1)

    def mod_w3_step(i):
        for k in range(4):
            ix = ((i % 2) * 4 + k, _rows(i // 2, 8))
            start(wmod_hbm.at[ix + (pl.ds(2 * M, 4 * M),)], wmb_v.at[ix], 0, 0)
            start(w3_hbm.at[ix], w3_v.at[ix], 1, 1)

    def w4_steps(lo, hi):
        for e in range(lo, hi):
            for queue, (blk, r) in enumerate(((e % 7, e // 7), (7 + e // 4, e % 4))):
                s, = [s for s, first, last in W4_PARTS if first <= blk < last]
                ix = (blk, pl.ds(32 * r, 32))
                start(w4_hbm.at[ix], w4_v.at[ix], s, queue)

    head_slot(0, low=1)
    _loop(1, 16, head_slot)
    start(c_hbm, c_v, 1, 0)
    start(x_hbm, x_v, 1, 1)
    _loop(0, 6, kv_slot)
    for buf in (c_v, x_v, wma_v, wq_v, wuk_v):
        wait(buf, 1)

    cond = c_v[...].astype(F32)
    cond = (cond * jax.nn.sigmoid(cond)).astype(BF)
    mod = _dot(cond, wma_v[...].reshape(M, 2 * M))
    shift_a, scale_a = mod[:, :M], mod[:, M:]
    x0 = x_v[...].astype(F32)
    h = (_ln(x0) * (1.0 + scale_a) + shift_a).astype(BF)

    _loop(6, 7, kv_slot)
    _gather_heads(wq_v, ta_v)
    _loop(7, 10, kv_slot)
    _gather_heads(wuk_v, tb_v)
    _loop(10, 13, kv_slot)

    def query(i):
        _loop(13 + i // 2, 13 + (i + 1) // 2, kv_slot)
        for j in range(4):
            s = 4 * i + j
            q = _dot(h, jnp.concatenate(_head_pair(ta_v, s), axis=1)).astype(BF)
            for e, wuk in enumerate(_head_pair(tb_v, s)):
                qa = lax.dot_general(q[:, e * D:(e + 1) * D], wuk, NT, preferred_element_type=F32)
                qa = qa * (D ** -0.5)
                for cb in range(4):
                    qa_v[cb, _rows(2 * s + e, B), :] = qa[:, cb * 128:(cb + 1) * 128]
    _loop(0, 4, query)
    _loop(15, LEAD, kv_slot)

    for b in range(B):
        qb_v[b] = jnp.concatenate([qa_v[cb, pl.ds(b, H, stride=B), :] for cb in range(4)], axis=1).astype(BF)
    m_v[...] = jnp.full(m_v.shape, -jnp.inf, F32)
    l_v[...] = jnp.zeros(l_v.shape, F32)
    acc_v[...] = jnp.zeros(acc_v.shape, F32)

    def attend(i, refill):
        sweep, b = i // B, i % B

        @pl.when(b == 0)
        def _():
            wait(kv_v.at[:, _rows(sweep, KC // 2)], sweep % 2)

        refill()
        kv = kv_v.at[_rows(b, 2), _rows(sweep, KC // 2)]
        s = lax.dot_general(qb_v[b], kv[...].reshape(KC, DC), NT, preferred_element_type=F32)
        m_old = m_v[b]
        m_new = jnp.maximum(m_old, jnp.max(s, axis=-1, keepdims=True))
        alpha = jnp.exp(m_old - m_new)
        p = jnp.exp(s - jnp.concatenate([m_new] * 4, axis=1))
        m_v[b] = m_new
        l_v[b] = alpha * l_v[b] + ((p[:, 0:128] + p[:, 128:256]) + (p[:, 256:384] + p[:, 384:512]))
        pv = _dot(p.astype(BF), kv[...].reshape(KC, DC))
        acc_v[b] = jnp.concatenate([alpha] * 4, axis=1) * acc_v[b] + pv
    _loop(0, NBLK - LEAD, lambda i: attend(i, lambda: kv_slot(i + LEAD)))
    _loop(NBLK - LEAD, NBLK, lambda i: attend(i, lambda: uv_o_slot(i - (NBLK - LEAD))))

    for b in range(B):
        latent = acc_v[b] / jnp.sum(l_v[b], axis=-1, keepdims=True)
        for cb in range(4):
            cc_v[cb, pl.ds(b, H, stride=B), :] = latent[:, cb * 128:(cb + 1) * 128]

    _loop(0, 6, mod_w3_step)
    wait(wuv_v, 2)
    _gather_heads(wuv_v, ta_v)
    _loop(6, 16, mod_w3_step)

    def value(i):
        for j in range(4):
            s = 4 * i + j
            for e, wuv in enumerate(_head_pair(ta_v, s)):
                latent = jnp.concatenate([cc_v[cb, _rows(2 * s + e, B), :] for cb in range(4)], axis=1)
                ctx_v[2 * s + e] = _dot(latent.astype(BF), wuv)
    _loop(0, 4, value)

    w4_steps(0, 4)
    wait(wo_v, 3)
    ctx = jnp.concatenate([ctx_v[i] for i in range(H)], axis=1).astype(BF)
    att = _dot(ctx, wo_v[...].reshape(H * D, M))

    w4_steps(4, 24)
    wait(wmb_v, 0)
    w4_steps(24, 28)
    mod = _dot(cond, wmb_v[...].reshape(M, 4 * M))
    gate_a, shift_b, scale_b, gate_b = (mod[:, i * M:(i + 1) * M] for i in range(4))
    x1 = x0 + gate_a * att

    y = _ln(x1) * (1.0 + scale_b) + shift_b
    yn = _ln(y).astype(BF)
    wait(w3_v, 1)
    g = jax.nn.gelu(_dot(yn, w3_v[...].reshape(M, F)), approximate=True).astype(BF)
    for s, first, last in W4_PARTS:
        wait(w4_v.at[pl.ds(first, last - first)], s)
        if first == 13: y, yb = jnp.zeros_like(y), x1 + gate_b * y
        y = y + _dot(g[:, first * 128:last * 128], w4_v[first:last].reshape((last - first) * 128, M))
    o_ref[...] = (yb + gate_b * y).astype(o_ref.dtype)


@jax.jit
def pallas_adaLN_cond__compressed_kv_cla__mixer_s_mlp__decode_kernel(
    A_x: jax.Array,
    A_c_kv: jax.Array,
    A_w_q: jax.Array,
    A_w_uk: jax.Array,
    A_w_uv: jax.Array,
    A_w_o: jax.Array,
    B_x: jax.Array,
    B_w1: jax.Array,
    B_w2: jax.Array,
    B_w3: jax.Array,
    B_w4: jax.Array,
    c: jax.Array,
    w_mod: jax.Array,
):
    assert A_x.shape == (B, 1, M) and A_c_kv.shape == (B, SK, DC) and B_w3.shape == (M, F)
    vmem = pltpu.VMEM
    out = pl.pallas_call(
        _kernel,
        out_shape=jax.ShapeDtypeStruct((B, M), A_x.dtype),
        in_specs=[pl.BlockSpec(memory_space=pltpu.HBM)] * 10,
        out_specs=pl.BlockSpec(memory_space=pltpu.VMEM),
        scratch_shapes=[
            vmem((2 * B, SK // 2, DC), BF),
            vmem((4, M * H // 4, D), BF), vmem((4, DC * H // 4, D), BF),
            vmem((4, DC * H // 4, D), BF), vmem((4, H * D // 4, M), BF),
            vmem((8, M // 8, F), BF), vmem((F // 128, 128, M), BF),
            vmem((8, M // 8, 2 * M), BF), vmem((8, M // 8, 4 * M), BF),
            vmem((B, M), BF), vmem((B, M), BF),
            vmem((16 * TS + 512, D), jnp.uint32), vmem((16 * TS + 512, D), jnp.uint32),
            vmem((4, (H + 1) * B, 128), F32), vmem((B, H, DC), BF),
            vmem((B, H, 128), F32), vmem((B, H, 128), F32), vmem((B, H, DC), F32),
            vmem((4, (H + 1) * B, 128), F32), vmem((H, B, D), F32),
            pltpu.SemaphoreType.DMA((4,)),
        ],
        compiler_params=pltpu.CompilerParams(vmem_limit_bytes=100 * 1024 * 1024, disable_semaphore_checks=True),
    )(
        A_x.reshape(B, M),
        A_c_kv.reshape(2 * B, SK // 2, DC),
        A_w_q.reshape(4, M * H // 4, D),
        A_w_uk.reshape(4, DC * H // 4, D),
        A_w_uv.reshape(4, DC * H // 4, D),
        A_w_o.reshape(4, H * D // 4, M),
        B_w3.reshape(8, M // 8, F),
        B_w4.reshape(F // 128, 128, M),
        c,
        w_mod.reshape(8, M // 8, 6 * M),
    )
    return out.reshape(B, 1, M)
```

```python
import jax
import jax.numpy as jnp
import numpy as np
from jax import lax
import jax.experimental.pallas as pl
import jax.experimental.pallas.tpu as pltpu

B, H, D, M, SK, DC, F = 8, 32, 128, 512, 4096, 512, 1792
BF, F32 = jnp.bfloat16, jnp.float32
NT = (((1,), (1,)), ((), ()))

KC = 512
NBLK = B * SK // KC
LEAD = 16
TS = 516
W4_PARTS = ((2, 0, 10), (3, 10, 13), (0, 13, 14))


def _ln(x):
    d = x - jnp.mean(x, axis=-1, keepdims=True)
    return d * lax.rsqrt(jnp.mean(d * d, axis=-1, keepdims=True) + 1e-5)


def _dot(a, b):
    return jnp.dot(a, b, preferred_element_type=F32)


def _rows(i, n):
    return pl.ds(pl.multiple_of(i * n, n), n)


def _loop(lo, hi, body):
    lax.fori_loop(lo, hi, lambda i, carry: (body(i), carry)[1], 0)


def _gather_heads(w_ref, t_ref):
    def step(i):
        words = pltpu.bitcast(w_ref[i // 4, _rows(i % 4, 32 * H), :], jnp.uint32)
        dst = t_ref.at[pl.ds(pl.multiple_of(32 * i, 32), 16 * TS + 32)]
        for r in range(32):
            dst[pl.ds(r, 16, stride=TS), :] = words[16 * r:16 * r + 16]
    _loop(0, 16, step)


def _head_pair(t_ref, s):
    w = t_ref[pl.ds(pl.multiple_of(s * TS, 4), 512), :]
    even = pltpu.bitcast(w << 16, F32).astype(BF)
    odd = pltpu.bitcast(w & np.uint32(0xFFFF0000), F32).astype(BF)
    return even, odd


def _kernel(x_hbm, kv_hbm, wq_hbm, wuk_hbm, wuv_hbm, wo_hbm, w3_hbm, w4_hbm, c_hbm, wmod_hbm, o_ref,
            kv_v, wq_v, wuk_v, wuv_v, wo_v, w3_v, w4_v, wma_v, wmb_v, x_v, c_v,
            ta_v, tb_v, qa_v, qb_v, m_v, l_v, acc_v, cc_v, ctx_v, sem):
    def start(src, dst, s, queue):
        pltpu.make_async_copy(src, dst, sem.at[s]).start(priority=queue)

    def wait(buf, s):
        pltpu.make_async_copy(buf, buf, sem.at[s]).wait()

    def head_slot(i, low=0):
        for k in range(4):
            for src, dst in ((wq_hbm, wq_v), (wuk_hbm, wuk_v)):
                for half in range(2):
                    ix = (pl.ds(2 * half, 2), _rows(4 * i + k, 64))
                    start(src.at[ix], dst.at[ix], 1, max(half, low))
            if k == 1:
                for e in range(2):
                    ix = ((i % 4) * 2 + e, _rows(i // 4, 16))
                    start(wmod_hbm.at[ix + (pl.ds(0, 2 * M),)], wma_v.at[ix], 1, max(e, low))

    def kv_slot(t):
        for u in range(16):
            ix = (pl.ds(2 * (u % B), 2), _rows(2 * t + u // B, 16))
            start(kv_hbm.at[ix], kv_v.at[ix], (t // B) % 2, u % 2)

    def uv_o_slot(i):
        for k in range(8):
            r, half = 4 * i + k // 2, pl.ds(2 * (k % 2), 2)
            start(wuv_hbm.at[half, _rows(r, 64)], wuv_v.at[half, _rows(r, 64)], 2, 0)
            start(wo_hbm.at[half, _rows(r, 16)], wo_v.at[half, _rows(r, 16)], 3, 1)

    def mod_w3_step(i):
        for k in range(4):
            ix = ((i % 2) * 4 + k, _rows(i // 2, 8))
            start(wmod_hbm.at[ix + (pl.ds(2 * M, 4 * M),)], wmb_v.at[ix], 0, 0)
            start(w3_hbm.at[ix], w3_v.at[ix], 1, 1)

    def w4_steps(lo, hi):
        for e in range(lo, hi):
            for queue, (blk, r) in enumerate(((e % 7, e // 7), (7 + e // 4, e % 4))):
                s, = [s for s, first, last in W4_PARTS if first <= blk < last]
                ix = (blk, pl.ds(32 * r, 32))
                start(w4_hbm.at[ix], w4_v.at[ix], s, queue)

    head_slot(0, low=1)
    _loop(1, 16, head_slot)
    start(c_hbm, c_v, 1, 0)
    start(x_hbm, x_v, 1, 1)
    _loop(0, 6, kv_slot)
    for buf in (c_v, x_v, wma_v, wq_v, wuk_v):
        wait(buf, 1)

    cond = c_v[...].astype(F32)
    cond = (cond * jax.nn.sigmoid(cond)).astype(BF)
    mod = _dot(cond, wma_v[...].reshape(M, 2 * M))
    shift_a, scale_a = mod[:, :M], mod[:, M:]
    x0 = x_v[...].astype(F32)
    h = (_ln(x0) * (1.0 + scale_a) + shift_a).astype(BF)

    _loop(6, 7, kv_slot)
    _gather_heads(wq_v, ta_v)
    _loop(7, 10, kv_slot)
    _gather_heads(wuk_v, tb_v)
    _loop(10, 13, kv_slot)

    def query(i):
        _loop(13 + i // 2, 13 + (i + 1) // 2, kv_slot)
        for j in range(4):
            s = 4 * i + j
            q = _dot(h, jnp.concatenate(_head_pair(ta_v, s), axis=1)).astype(BF)
            for e, wuk in enumerate(_head_pair(tb_v, s)):
                qa = lax.dot_general(q[:, e * D:(e + 1) * D], wuk, NT, preferred_element_type=F32)
                qa = qa * (D ** -0.5)
                for cb in range(4):
                    qa_v[cb, _rows(2 * s + e, B), :] = qa[:, cb * 128:(cb + 1) * 128]
    _loop(0, 4, query)
    _loop(15, LEAD, kv_slot)

    for b in range(B):
        qb_v[b] = jnp.concatenate([qa_v[cb, pl.ds(b, H, stride=B), :] for cb in range(4)], axis=1).astype(BF)
    m_v[...] = jnp.full(m_v.shape, -jnp.inf, F32)
    l_v[...] = jnp.zeros(l_v.shape, F32)
    acc_v[...] = jnp.zeros(acc_v.shape, F32)

    def attend(i, refill):
        sweep, b = i // B, i % B

        @pl.when(b == 0)
        def _():
            wait(kv_v.at[:, _rows(sweep, KC // 2)], sweep % 2)

        refill()
        kv = kv_v.at[_rows(b, 2), _rows(sweep, KC // 2)]
        s = lax.dot_general(qb_v[b], kv[...].reshape(KC, DC), NT, preferred_element_type=F32)
        m_old = m_v[b]
        m_new = jnp.maximum(m_old, jnp.max(s, axis=-1, keepdims=True))
        alpha = jnp.exp(m_old - m_new)
        p = jnp.exp(s - jnp.concatenate([m_new] * 4, axis=1))
        m_v[b] = m_new
        l_v[b] = alpha * l_v[b] + ((p[:, 0:128] + p[:, 128:256]) + (p[:, 256:384] + p[:, 384:512]))
        pv = _dot(p.astype(BF), kv[...].reshape(KC, DC))
        acc_v[b] = jnp.concatenate([alpha] * 4, axis=1) * acc_v[b] + pv
    _loop(0, NBLK - LEAD, lambda i: attend(i, lambda: kv_slot(i + LEAD)))
    _loop(NBLK - LEAD, NBLK, lambda i: attend(i, lambda: uv_o_slot(i - (NBLK - LEAD))))

    for b in range(B):
        latent = acc_v[b] / jnp.sum(l_v[b], axis=-1, keepdims=True)
        for cb in range(4):
            cc_v[cb, pl.ds(b, H, stride=B), :] = latent[:, cb * 128:(cb + 1) * 128]

    _loop(0, 6, mod_w3_step)
    wait(wuv_v, 2)
    _gather_heads(wuv_v, ta_v)
    _loop(6, 16, mod_w3_step)

    def value(i):
        for j in range(4):
            s = 4 * i + j
            for e, wuv in enumerate(_head_pair(ta_v, s)):
                latent = jnp.concatenate([cc_v[cb, _rows(2 * s + e, B), :] for cb in range(4)], axis=1)
                ctx_v[2 * s + e] = _dot(latent.astype(BF), wuv)
    _loop(0, 4, value)

    w4_steps(0, 4)
    wait(wo_v, 3)
    ctx = jnp.concatenate([ctx_v[i] for i in range(H)], axis=1).astype(BF)
    att = _dot(ctx, wo_v[...].reshape(H * D, M))

    w4_steps(4, 24)
    wait(wmb_v, 0)
    w4_steps(24, 28)
    mod = _dot(cond, wmb_v[...].reshape(M, 4 * M))
    gate_a, shift_b, scale_b, gate_b = (mod[:, i * M:(i + 1) * M] for i in range(4))
    x1 = x0 + gate_a * att

    y = _ln(x1) * (1.0 + scale_b) + shift_b
    yn = _ln(y).astype(BF)
    wait(w3_v, 1)
    g = jax.nn.gelu(_dot(yn, w3_v[...].reshape(M, F)), approximate=True).astype(BF)
    out = x1 + gate_b * y
    for s, first, last in W4_PARTS:
        wait(w4_v.at[pl.ds(first, last - first)], s)
        w4 = w4_v[first:last].reshape((last - first) * 128, M)
        out = out + gate_b * _dot(g[:, first * 128:last * 128], w4)
    o_ref[...] = out.astype(o_ref.dtype)


@jax.jit
def pallas_adaLN_cond__compressed_kv_cla__mixer_s_mlp__decode_kernel(
    A_x: jax.Array,
    A_c_kv: jax.Array,
    A_w_q: jax.Array,
    A_w_uk: jax.Array,
    A_w_uv: jax.Array,
    A_w_o: jax.Array,
    B_x: jax.Array,
    B_w1: jax.Array,
    B_w2: jax.Array,
    B_w3: jax.Array,
    B_w4: jax.Array,
    c: jax.Array,
    w_mod: jax.Array,
):
    assert A_x.shape == (B, 1, M) and A_c_kv.shape == (B, SK, DC) and B_w3.shape == (M, F)
    vmem = pltpu.VMEM
    out = pl.pallas_call(
        _kernel,
        out_shape=jax.ShapeDtypeStruct((B, M), A_x.dtype),
        in_specs=[pl.BlockSpec(memory_space=pltpu.HBM)] * 10,
        out_specs=pl.BlockSpec(memory_space=pltpu.VMEM),
        scratch_shapes=[
            vmem((2 * B, SK // 2, DC), BF),
            vmem((4, M * H // 4, D), BF), vmem((4, DC * H // 4, D), BF),
            vmem((4, DC * H // 4, D), BF), vmem((4, H * D // 4, M), BF),
            vmem((8, M // 8, F), BF), vmem((F // 128, 128, M), BF),
            vmem((8, M // 8, 2 * M), BF), vmem((8, M // 8, 4 * M), BF),
            vmem((B, M), BF), vmem((B, M), BF),
            vmem((16 * TS + 512, D), jnp.uint32), vmem((16 * TS + 512, D), jnp.uint32),
            vmem((4, (H + 1) * B, 128), F32), vmem((B, H, DC), BF),
            vmem((B, H, 128), F32), vmem((B, H, 128), F32), vmem((B, H, DC), F32),
            vmem((4, (H + 1) * B, 128), F32), vmem((H, B, D), F32),
            pltpu.SemaphoreType.DMA((4,)),
        ],
        compiler_params=pltpu.CompilerParams(vmem_limit_bytes=100 * 1024 * 1024, disable_semaphore_checks=True),
    )(
        A_x.reshape(B, M),
        A_c_kv.reshape(2 * B, SK // 2, DC),
        A_w_q.reshape(4, M * H // 4, D),
        A_w_uk.reshape(4, DC * H // 4, D),
        A_w_uv.reshape(4, DC * H // 4, D),
        A_w_o.reshape(4, H * D // 4, M),
        B_w3.reshape(8, M // 8, F),
        B_w4.reshape(F // 128, 128, M),
        c,
        w_mod.reshape(8, M // 8, 6 * M),
    )
    return out.reshape(B, 1, M)
```

```python
import jax
import jax.numpy as jnp
import numpy as np
from jax import lax
import jax.experimental.pallas as pl
import jax.experimental.pallas.tpu as pltpu

B, H, D, M, SK, DC, F = 8, 32, 128, 512, 4096, 512, 1792
BF, F32 = jnp.bfloat16, jnp.float32
NT = (((1,), (1,)), ((), ()))

KC = 512
NBLK = B * SK // KC
LEAD = 16
TS = 516
W4_PARTS = ((2, 0, 10), (3, 10, 13), (0, 13, 14))


def _ln(x):
    d = x - jnp.mean(x, axis=-1, keepdims=True)
    return d * lax.rsqrt(jnp.mean(d * d, axis=-1, keepdims=True) + 1e-5)


def _dot(a, b):
    return jnp.dot(a, b, preferred_element_type=F32)


def _rows(i, n):
    return pl.ds(pl.multiple_of(i * n, n), n)


def _loop(lo, hi, body):
    lax.fori_loop(lo, hi, lambda i, carry: (body(i), carry)[1], 0)


def _gather_heads(w_ref, t_ref):
    def step(i):
        words = pltpu.bitcast(w_ref[i >> 2, _rows(i & 3, 32 * H), :], jnp.uint32)
        dst = t_ref.at[pl.ds(pl.multiple_of(32 * i, 32), 16 * TS + 32)]
        for r in range(32):
            dst[pl.ds(r, 16, stride=TS), :] = words[16 * r:16 * r + 16]
    _loop(0, 16, step)


def _head_pair(t_ref, s):
    w = t_ref[pl.ds(pl.multiple_of(s * TS, 4), 512), :]
    even = pltpu.bitcast(w << 16, F32).astype(BF)
    odd = pltpu.bitcast(w & np.uint32(0xFFFF0000), F32).astype(BF)
    return even, odd


def _kernel(x_hbm, kv_hbm, wq_hbm, wuk_hbm, wuv_hbm, wo_hbm, w3_hbm, w4_hbm, c_hbm, wmod_hbm, o_ref,
            kv_v, wq_v, wuk_v, wuv_v, wo_v, w3_v, w4_v, wma_v, wmb_v, x_v, c_v,
            ta_v, tb_v, qa_v, qb_v, m_v, l_v, acc_v, cc_v, ctx_v, sem):
    def start(src, dst, s, queue):
        pltpu.make_async_copy(src, dst, sem.at[s]).start(priority=queue)

    def wait(buf, s):
        pltpu.make_async_copy(buf, buf, sem.at[s]).wait()

    def head_slot(i, low=0):
        for k in range(4):
            for src, dst in ((wq_hbm, wq_v), (wuk_hbm, wuk_v)):
                for half in range(2):
                    ix = (pl.ds(2 * half, 2), _rows(4 * i + k, 64))
                    start(src.at[ix], dst.at[ix], 1, max(half, low))
            if k == 1:
                for e in range(2):
                    ix = ((i & 3) * 2 + e, _rows(i >> 2, 16))
                    start(wmod_hbm.at[ix + (pl.ds(0, 2 * M),)], wma_v.at[ix], 1, max(e, low))

    def kv_slot(t):
        for u in range(16):
            ix = (pl.ds(2 * (u % B), 2), _rows(2 * t + u // B, 16))
            start(kv_hbm.at[ix], kv_v.at[ix], (t >> 3) & 1, u % 2)

    def uv_o_slot(i):
        for k in range(8):
            r, half = 4 * i + k // 2, pl.ds(2 * (k % 2), 2)
            start(wuv_hbm.at[half, _rows(r, 64)], wuv_v.at[half, _rows(r, 64)], 2, 0)
            start(wo_hbm.at[half, _rows(r, 16)], wo_v.at[half, _rows(r, 16)], 3, 1)

    def mod_w3_step(i):
        for k in range(4):
            ix = ((i & 1) * 4 + k, _rows(i >> 1, 8))
            start(wmod_hbm.at[ix + (pl.ds(2 * M, 4 * M),)], wmb_v.at[ix], 0, 0)
            start(w3_hbm.at[ix], w3_v.at[ix], 1, 1)

    def w4_steps(lo, hi):
        for e in range(lo, hi):
            for queue, (blk, r) in enumerate(((e % 7, e // 7), (7 + e // 4, e % 4))):
                s, = [s for s, first, last in W4_PARTS if first <= blk < last]
                ix = (blk, pl.ds(32 * r, 32))
                start(w4_hbm.at[ix], w4_v.at[ix], s, queue)

    head_slot(0, low=1)
    _loop(1, 16, head_slot)
    start(c_hbm, c_v, 1, 0)
    start(x_hbm, x_v, 1, 1)
    _loop(0, 6, kv_slot)
    for buf in (c_v, x_v, wma_v, wq_v, wuk_v):
        wait(buf, 1)

    cond = c_v[...].astype(F32)
    cond = (cond * jax.nn.sigmoid(cond)).astype(BF)
    mod = _dot(cond, wma_v[...].reshape(M, 2 * M))
    shift_a, scale_a = mod[:, :M], mod[:, M:]
    x0 = x_v[...].astype(F32)
    h = (_ln(x0) * (1.0 + scale_a) + shift_a).astype(BF)

    _loop(6, 7, kv_slot)
    _gather_heads(wq_v, ta_v)
    _loop(7, 10, kv_slot)
    _gather_heads(wuk_v, tb_v)
    _loop(10, 13, kv_slot)

    def query(i):
        _loop(13 + (i >> 1), 13 + ((i + 1) >> 1), kv_slot)
        for j in range(4):
            s = 4 * i + j
            q = _dot(h, jnp.concatenate(_head_pair(ta_v, s), axis=1)).astype(BF)
            for e, wuk in enumerate(_head_pair(tb_v, s)):
                qa = lax.dot_general(q[:, e * D:(e + 1) * D], wuk, NT, preferred_element_type=F32)
                qa = qa * (D ** -0.5)
                for cb in range(4):
                    qa_v[cb, _rows(2 * s + e, B), :] = qa[:, cb * 128:(cb + 1) * 128]
    _loop(0, 4, query)
    _loop(15, LEAD, kv_slot)

    for b in range(B):
        qb_v[b] = jnp.concatenate([qa_v[cb, pl.ds(b, H, stride=B), :] for cb in range(4)], axis=1).astype(BF)
    m_v[...] = jnp.full(m_v.shape, -jnp.inf, F32)
    l_v[...] = jnp.zeros(l_v.shape, F32)
    acc_v[...] = jnp.zeros(acc_v.shape, F32)

    def attend(i, refill):
        sweep, b = i >> 3, i & 7

        @pl.when(b == 0)
        def _():
            wait(kv_v.at[:, _rows(sweep, KC // 2)], sweep & 1)

        refill()
        kv = kv_v.at[_rows(b, 2), _rows(sweep, KC // 2)]
        s = lax.dot_general(qb_v[b], kv[...].reshape(KC, DC), NT, preferred_element_type=F32)
        m_old = m_v[b]
        m_new = jnp.maximum(m_old, jnp.max(s, axis=-1, keepdims=True))
        alpha = jnp.exp(m_old - m_new)
        p = jnp.exp(s - jnp.concatenate([m_new] * 4, axis=1))
        m_v[b] = m_new
        l_v[b] = alpha * l_v[b] + ((p[:, 0:128] + p[:, 128:256]) + (p[:, 256:384] + p[:, 384:512]))
        pv = _dot(p.astype(BF), kv[...].reshape(KC, DC))
        acc_v[b] = jnp.concatenate([alpha] * 4, axis=1) * acc_v[b] + pv
    _loop(0, NBLK - LEAD, lambda i: attend(i, lambda: kv_slot(i + LEAD)))
    _loop(NBLK - LEAD, NBLK, lambda i: attend(i, lambda: uv_o_slot(i - (NBLK - LEAD))))

    for b in range(B):
        latent = acc_v[b] / jnp.sum(l_v[b], axis=-1, keepdims=True)
        for cb in range(4):
            cc_v[cb, pl.ds(b, H, stride=B), :] = latent[:, cb * 128:(cb + 1) * 128]

    _loop(0, 6, mod_w3_step)
    wait(wuv_v, 2)
    _gather_heads(wuv_v, ta_v)
    _loop(6, 16, mod_w3_step)

    def value(i):
        for j in range(4):
            s = 4 * i + j
            for e, wuv in enumerate(_head_pair(ta_v, s)):
                latent = jnp.concatenate([cc_v[cb, _rows(2 * s + e, B), :] for cb in range(4)], axis=1)
                ctx_v[2 * s + e] = _dot(latent.astype(BF), wuv)
    _loop(0, 4, value)

    w4_steps(0, 4)
    wait(wo_v, 3)
    ctx = jnp.concatenate([ctx_v[i] for i in range(H)], axis=1).astype(BF)
    att = _dot(ctx, wo_v[...].reshape(H * D, M))

    w4_steps(4, 24)
    wait(wmb_v, 0)
    w4_steps(24, 28)
    mod = _dot(cond, wmb_v[...].reshape(M, 4 * M))
    gate_a, shift_b, scale_b, gate_b = (mod[:, i * M:(i + 1) * M] for i in range(4))
    x1 = x0 + gate_a * att

    y = _ln(x1) * (1.0 + scale_b) + shift_b
    yn = _ln(y).astype(BF)
    wait(w3_v, 1)
    g = jax.nn.gelu(_dot(yn, w3_v[...].reshape(M, F)), approximate=True).astype(BF)
    out = x1 + gate_b * y
    for s, first, last in W4_PARTS:
        wait(w4_v.at[pl.ds(first, last - first)], s)
        w4 = w4_v[first:last].reshape((last - first) * 128, M)
        out = out + gate_b * _dot(g[:, first * 128:last * 128], w4)
    o_ref[...] = out.astype(o_ref.dtype)


@jax.jit
def pallas_adaLN_cond__compressed_kv_cla__mixer_s_mlp__decode_kernel(
    A_x: jax.Array,
    A_c_kv: jax.Array,
    A_w_q: jax.Array,
    A_w_uk: jax.Array,
    A_w_uv: jax.Array,
    A_w_o: jax.Array,
    B_x: jax.Array,
    B_w1: jax.Array,
    B_w2: jax.Array,
    B_w3: jax.Array,
    B_w4: jax.Array,
    c: jax.Array,
    w_mod: jax.Array,
):
    assert A_x.shape == (B, 1, M) and A_c_kv.shape == (B, SK, DC) and B_w3.shape == (M, F)
    vmem = pltpu.VMEM
    out = pl.pallas_call(
        _kernel,
        out_shape=jax.ShapeDtypeStruct((B, M), A_x.dtype),
        in_specs=[pl.BlockSpec(memory_space=pltpu.HBM)] * 10,
        out_specs=pl.BlockSpec(memory_space=pltpu.VMEM),
        scratch_shapes=[
            vmem((2 * B, SK // 2, DC), BF),
            vmem((4, M * H // 4, D), BF), vmem((4, DC * H // 4, D), BF),
            vmem((4, DC * H // 4, D), BF), vmem((4, H * D // 4, M), BF),
            vmem((8, M // 8, F), BF), vmem((F // 128, 128, M), BF),
            vmem((8, M // 8, 2 * M), BF), vmem((8, M // 8, 4 * M), BF),
            vmem((B, M), BF), vmem((B, M), BF),
            vmem((16 * TS + 512, D), jnp.uint32), vmem((16 * TS + 512, D), jnp.uint32),
            vmem((4, (H + 1) * B, 128), F32), vmem((B, H, DC), BF),
            vmem((B, H, 128), F32), vmem((B, H, 128), F32), vmem((B, H, DC), F32),
            vmem((4, (H + 1) * B, 128), F32), vmem((H, B, D), F32),
            pltpu.SemaphoreType.DMA((4,)),
        ],
        compiler_params=pltpu.CompilerParams(vmem_limit_bytes=100 * 1024 * 1024, disable_semaphore_checks=True),
    )(
        A_x.reshape(B, M),
        A_c_kv.reshape(2 * B, SK // 2, DC),
        A_w_q.reshape(4, M * H // 4, D),
        A_w_uk.reshape(4, DC * H // 4, D),
        A_w_uv.reshape(4, DC * H // 4, D),
        A_w_o.reshape(4, H * D // 4, M),
        B_w3.reshape(8, M // 8, F),
        B_w4.reshape(F // 128, 128, M),
        c,
        w_mod.reshape(8, M // 8, 6 * M),
    )
    return out.reshape(B, 1, M)
```
